```python
import jax
import jax.numpy as jnp

def _softmax(x, axis=-1):
    return jax.nn.softmax(x, axis=axis)
def _gelu(x):
    return jax.nn.gelu(x, approximate=True)
def _silu(x):
    return jax.nn.silu(x)
def _sigmoid(x):
    return jax.nn.sigmoid(x)
def _layernorm(x, axis=-1, eps=1e-5):
    m = jnp.mean(x, axis=axis, keepdims=True)
    v = jnp.var(x, axis=axis, keepdims=True)
    return (x - m) / jnp.sqrt(v + eps)
def _scatter_add(tgt, idx, src, axis=0):
    return tgt.at[idx].add(src)
def _segment_sum(src, seg, n):
    return jax.ops.segment_sum(src, seg, n)
class _Rng:
    def __init__(self, key):
        self._k = key
    def _next(self):
        self._k, sub = jax.random.split(self._k)
        return sub
    def normal(self, shape):
        return jax.random.normal(self._next(), shape, dtype=jnp.bfloat16)
    def randint(self, lo, hi, shape):
        return jax.random.randint(self._next(), shape, lo, hi, dtype=jnp.int32)
    def uniform(self, shape, lo=0.0, hi=1.0):
        return jax.random.uniform(self._next(), shape, jnp.bfloat16, lo, hi)
    def permutation(self, n):
        return jax.random.permutation(self._next(), n)


kernel_name = 'interleave_layers__sliding_block__moe_arch_mod__prompt'

def setup_inputs():
    _rng = _Rng(jax.random.key(int.from_bytes(__import__("os").urandom(4), "little")))
    _w = (lambda a: (lambda t: t.astype(jnp.bfloat16) if jnp.issubdtype(t.dtype, jnp.floating) else t)(jnp.asarray(a)))
    def _A_setup():
        B, S, D = 1, 2048, 1024
        return {
            "x": _w((lambda *s: _rng.normal(s) * 0.05)(B, S, D)),
            "wqkv": _w((lambda *s: _rng.normal(s) * 0.05)(D, 3 * D)),
            "wo": _w((lambda *s: _rng.normal(s) * 0.05)(D, D)),
        }
    _A_in = _A_setup()

    def _B_setup():
        B, S, D, F, C = 1, 2048, 1024, 3584, 1
        return {
            "x": _w((lambda *s: _rng.normal(s) * 0.05)(B, S, D)),
            "w_r": _w((lambda *s: _rng.normal(s) * 0.05)(D)),
            "w_gate": _w((lambda *s: _rng.normal(s) * 0.05)(D, F)),
            "w_up": _w((lambda *s: _rng.normal(s) * 0.05)(D, F)),
            "w_down": _w((lambda *s: _rng.normal(s) * 0.05)(F, D)),
        }
    _B_in = _B_setup()

    return {
        "A_x": _A_in["x"],
        "A_wqkv": _A_in["wqkv"],
        "A_wo": _A_in["wo"],
        "B_x": _B_in["x"],
        "B_w_r": _B_in["w_r"],
        "B_w_gate": _B_in["w_gate"],
        "B_w_up": _B_in["w_up"],
        "B_w_down": _B_in["w_down"],
    }

def reference(A_x, A_wqkv, A_wo, B_x, B_w_r, B_w_gate, B_w_up, B_w_down):
    def _A_ref(x, wqkv, wo):
        B, S, D = x.shape
        H = 32; Dh = D // H; W = 256
        qkv = (lambda x, *d: x.transpose(*d))((x @ wqkv).reshape(B, S, 3, H, Dh), 2, 0, 3, 1, 4)
        q, k, v = qkv[0], qkv[1], qkv[2]
        scores = jnp.einsum("bhqd,bhkd->bhqk", q, k) * (Dh ** -0.5)
        idx = jnp.arange(S)
        mask = (idx[:, None] - idx[None, :] >= 0) & (idx[:, None] - idx[None, :] < W)
        scores = jnp.where(mask[None, None], scores, -1e9)
        p = _softmax(scores, axis=-1)
        o = jnp.einsum("bhqk,bhkd->bhqd", p, v)
        return (lambda x, *d: x.transpose(*d))(o, 0, 2, 1, 3).reshape(B, S, D) @ wo

    def _B_ref(x, w_r, w_gate, w_up, w_down):
        B, S, D = x.shape
        C = 1
        r = x @ w_r
        idx = jnp.argsort(-r, axis=-1)[:, :C]
        idx_e = jnp.repeat(idx.reshape(B, C, 1), D, axis=2)
        x_sel = jnp.take_along_axis(x, idx_e, axis=1)
        g = _silu(x_sel @ w_gate)
        u = x_sel @ w_up
        y = (g * u) @ w_down
        r_sel = _sigmoid(jnp.take_along_axis(r, idx, axis=1))
        y = y * r_sel.reshape(B, C, 1)
        b_off = (jnp.arange(B) * S).reshape(B, 1)
        flat_idx = (idx + b_off).reshape(B * C)
        zero = (x * 0.0).reshape(B * S, D)
        upd = _scatter_add(zero, flat_idx, y.reshape(B * C, D), axis=0)
        return x + upd.reshape(B, S, D)

    x = A_x
    x = x + _A_ref(_layernorm(x, axis=-1), A_wqkv, A_wo)
    x = x + _B_ref(_layernorm(x, axis=-1), B_w_r, B_w_gate, B_w_up, B_w_down)
    x = x + _A_ref(_layernorm(x, axis=-1), A_wqkv, A_wo)
    x = x + _B_ref(_layernorm(x, axis=-1), B_w_r, B_w_gate, B_w_up, B_w_down)
    return x
```

```python
import functools
import numpy as np
import jax
import jax.numpy as jnp
from jax import lax
from jax.experimental import pallas as pl
from jax.experimental.pallas import tpu as pltpu

S, D, F = 2048, 1024, 3584
H, DH, W = 32, 32, 256
R = 256
NB = S // R
G = D // 128
RC = R // G
KB = 32
f32, bf16 = jnp.float32, jnp.bfloat16
LOG2E = 1.4426950408889634
SCALE = 0.1767578125
EPS = float(np.float32(1e-5).astype(bf16))
NEG = -1e9 * LOG2E


def rb(x):
    return x.astype(bf16).astype(f32)


def layernorm(x):
    m = jnp.sum(x, axis=-1, keepdims=True) * (1.0 / D)
    c = x - m
    v = jnp.sum(c * c, axis=-1, keepdims=True) * (1.0 / D)
    s = rb(jnp.sqrt(rb(rb(v) + EPS)))
    return rb(x - rb(m)) * (1.0 / s)


def kernel(x_hbm, wqkv_hbm, wo_hbm, wr_ref, wg_hbm, wu_hbm, wd_hbm, out_hbm,
           x_buf, x1_buf, h_buf, q_buf, k_buf, v_buf, o_buf, wqkv_buf, wo_buf,
           wg_buf, wu_buf, wd_buf, best_ref, sem_x, sem_w, sem_o):
    def x_copy(b):
        return pltpu.make_async_copy(x_hbm.at[pl.ds(b * R, R)], x_buf.at[pl.ds(b * R, R)], sem_x.at[b])

    def out_copy(b):
        return pltpu.make_async_copy(x_buf.at[pl.ds(b * R, R)], out_hbm.at[pl.ds(b * R, R)], sem_o.at[b])

    w_copies = [
        pltpu.make_async_copy(wqkv_hbm, wqkv_buf, sem_w.at[0]),
        pltpu.make_async_copy(wo_hbm, wo_buf, sem_w.at[1]),
        pltpu.make_async_copy(wg_hbm, wg_buf, sem_w.at[2]),
        pltpu.make_async_copy(wu_hbm, wu_buf, sem_w.at[3]),
        pltpu.make_async_copy(wd_hbm, wd_buf, sem_w.at[4]),
    ]
    x_copy(0).start()
    w_copies[0].start()
    for b in range(1, NB):
        x_copy(b).start()
    for c in w_copies[1:]:
        c.start()

    lane = lax.broadcasted_iota(jnp.int32, (KB, 128), 1)
    row = lax.broadcasted_iota(jnp.int32, (KB, 128), 0)

    def rows_of(b, n=R, off=0):
        return pl.ds(pl.multiple_of(b * R + off, RC), n)

    def cols_of(g):
        return pl.ds(pl.multiple_of(g * 128, 128), 128)

    def ln_stage(b, g):
        rr = rows_of(b, RC, g * RC)
        h_buf[rr, :] = layernorm(x_buf[rr, :].astype(f32)).astype(bf16)

    def qkv_stage(b, g):
        rr = rows_of(b)
        h = h_buf[rr, :]
        q = jnp.dot(h, wqkv_buf[:, cols_of(g)], preferred_element_type=f32)
        q_buf[g, rr, :] = (q * (SCALE * LOG2E)).astype(bf16)
        k = jnp.dot(h, wqkv_buf[:, cols_of(g + G)], preferred_element_type=f32)
        k_buf[g, rr, :] = k.astype(bf16)
        v = jnp.dot(h, wqkv_buf[:, cols_of(g + 2 * G)], preferred_element_type=f32)
        v_buf[g, rr, :] = v.astype(bf16)

    def blockdiag(t):
        z = jnp.zeros_like(t)
        return jnp.concatenate([jnp.where(lane // DH == hh, t, z) for hh in range(4)], axis=0)

    def segment(x, op, fill):
        ln = lane[: x.shape[0]] // DH
        out = None
        for hh in range(4):
            r = op(jnp.where(ln == hh, x, fill), axis=-1, keepdims=True)
            out = r if out is None else jnp.where(ln == hh, r, out)
        return out

    def att_stage(b, g, first):
        nt = R // KB
        us = list(range(nt if first else 0, 2 * nt))
        lo = {u: max(0, u - nt) for u in us}
        hi = {u: min(nt, u + 1) for u in us}
        q = q_buf[g, rows_of(b), :]
        s = {}
        for u in us:
            kt = k_buf[g, rows_of(b, KB, (u - nt) * KB), :]
            su = lax.dot_general(q[lo[u] * KB: hi[u] * KB], blockdiag(kt),
                                 (((1,), (1,)), ((), ())), preferred_element_type=f32)
            for i in range(lo[u], hi[u]):
                t = su[(i - lo[u]) * KB: (i - lo[u] + 1) * KB]
                if u == i:
                    t = jnp.where(lane % KB > row, t, NEG)
                elif u == i + nt:
                    t = jnp.where(lane % KB <= row, t, NEG)
                s[u, i] = t
        p = {}
        linv = {}
        for i in range(nt):
            mine = [u for u in us if lo[u] <= i < hi[u]]
            m = functools.reduce(jnp.maximum, [s[u, i] for u in mine])
            m = segment(m, jnp.max, -np.inf)
            e = [jnp.exp2(s[u, i] - m) for u in mine]
            l = segment(functools.reduce(jnp.add, e), jnp.sum, 0.0)
            linv[i] = 1.0 / l
            for u, eu in zip(mine, e):
                p[u, i] = eu.astype(bf16)
        acc = {}
        for u in us:
            vt = v_buf[g, rows_of(b, KB, (u - nt) * KB), :]
            pu = jnp.concatenate([p[u, i] for i in range(lo[u], hi[u])], axis=0)
            ou = jnp.dot(pu, blockdiag(vt), preferred_element_type=f32)
            for i in range(lo[u], hi[u]):
                t = ou[(i - lo[u]) * KB: (i - lo[u] + 1) * KB]
                acc[i] = t if i not in acc else acc[i] + t
        o = jnp.concatenate([acc[i] * linv[i] for i in range(nt)], axis=0)
        o_buf[rows_of(b), cols_of(g)] = o.astype(bf16)

    def out_stage(b, g):
        rr = rows_of(b)
        a = jnp.dot(o_buf[rr, :], wo_buf[:, cols_of(g)], preferred_element_type=f32)
        x1_buf[rr, cols_of(g)] = (x_buf[rr, cols_of(g)].astype(f32) + rb(a)).astype(bf16)

    def router(h1):
        return rb(jnp.sum(h1 * wr_ref[...].astype(f32), axis=-1, keepdims=True))

    def epi_stage(b, g):
        rr = rows_of(b, RC, g * RC)
        x1 = x1_buf[rr, :].astype(f32)
        h1 = rb(layernorm(x1))
        x_buf[rr, :] = (x1 + h1).astype(bf16)
        r = jnp.broadcast_to(router(h1), (RC, 128))
        gt = r > best_ref[0]
        best_ref[0] = jnp.where(gt, r, best_ref[0])
        best_ref[1] = jnp.where(gt, (row + (b * R + g * RC)).astype(f32), best_ref[1])

    def steps(*stages):
        def body(g, _):
            for st in stages:
                st(g)
        lax.fori_loop(0, G, body, None)

    P = functools.partial

    def layer(li, _):
        best_ref[0] = jnp.full((RC, 128), -np.inf, f32)
        best_ref[1] = jnp.zeros((RC, 128), f32)

        def wait_x(b):
            @pl.when(li == 0)
            def _():
                x_copy(b).wait()

        def send(b):
            @pl.when(li == 1)
            def _():
                out_copy(b).start()

        wait_x(0)
        steps(P(ln_stage, 0))
        wait_x(1)

        @pl.when(li == 0)
        def _():
            w_copies[0].wait()
        steps(P(qkv_stage, 0), P(ln_stage, 1))
        wait_x(2)
        steps(P(att_stage, 0, first=True), P(qkv_stage, 1), P(ln_stage, 2))
        wait_x(3)

        @pl.when(li == 0)
        def _():
            w_copies[1].wait()
        steps(P(out_stage, 0), P(att_stage, 1, first=False), P(qkv_stage, 2), P(ln_stage, 3))

        def steady(b, _):
            wait_x(b + 2)
            steps(P(epi_stage, b - 2), P(out_stage, b - 1), P(att_stage, b, first=False),
                  P(qkv_stage, b + 1), P(ln_stage, b + 2))
            send(b - 2)
        lax.fori_loop(2, NB - 2, steady, None)
        b = NB - 2
        steps(P(epi_stage, b - 2), P(out_stage, b - 1), P(att_stage, b, first=False), P(qkv_stage, b + 1))
        send(b - 2)
        b = NB - 1
        steps(P(epi_stage, b - 2), P(out_stage, b - 1), P(att_stage, b, first=False))
        send(b - 2)
        steps(P(epi_stage, NB - 2), P(out_stage, NB - 1))
        send(NB - 2)
        steps(P(epi_stage, NB - 1))
        send(NB - 1)

        bv = best_ref[0]
        idx = jnp.min(jnp.where(bv == jnp.max(bv), best_ref[1], float(S - 1))).astype(jnp.int32)
        t0 = pl.multiple_of((idx // 16) * 16, 16)
        tt = pl.ds(t0, 16)

        @pl.when(li == 0)
        def _():
            for c in w_copies[2:]:
                c.wait()
        x1 = x1_buf[tt, :].astype(f32)
        h1 = rb(layernorm(x1))
        hb = h1.astype(bf16)
        gt = rb(jnp.dot(hb, wg_buf[...], preferred_element_type=f32))
        gt = rb(gt * jax.nn.sigmoid(gt))
        up = rb(jnp.dot(hb, wu_buf[...], preferred_element_type=f32))
        y = rb(jnp.dot((gt * up).astype(bf16), wd_buf[...], preferred_element_type=f32))
        y = rb(y * rb(jax.nn.sigmoid(router(h1))))
        sel = lax.broadcasted_iota(jnp.int32, (16, D), 0) == idx - t0
        new = (x1 + jnp.where(sel, rb(h1 + y), h1)).astype(bf16)

        @pl.when(li == 1)
        def _():
            for b in range(NB):
                out_copy(b).wait()
        x_buf[tt, :] = new

        @pl.when(li == 1)
        def _():
            c = pltpu.make_async_copy(x_buf.at[tt], out_hbm.at[tt], sem_o.at[0])
            c.start()
            c.wait()

    lax.fori_loop(0, 2, layer, None)


@jax.jit
def pallas_interleave_layers__sliding_block__moe_arch_mod__prompt_kernel(
    A_x, A_wqkv, A_wo, B_x, B_w_r, B_w_gate, B_w_up, B_w_down,
):
    any_spec = pl.BlockSpec(memory_space=pl.ANY)
    out = pl.pallas_call(
        kernel,
        out_shape=jax.ShapeDtypeStruct((S, D), bf16),
        in_specs=[any_spec, any_spec, any_spec, pl.BlockSpec(memory_space=pltpu.VMEM),
                  any_spec, any_spec, any_spec],
        out_specs=any_spec,
        scratch_shapes=[
            pltpu.VMEM((S, D), bf16),
            pltpu.VMEM((S, D), bf16),
            pltpu.VMEM((S, D), bf16),
            pltpu.VMEM((G, S, 128), bf16),
            pltpu.VMEM((G, S, 128), bf16),
            pltpu.VMEM((G, S, 128), bf16),
            pltpu.VMEM((S, D), bf16),
            pltpu.VMEM((D, 3 * D), bf16),
            pltpu.VMEM((D, D), bf16),
            pltpu.VMEM((D, F), bf16),
            pltpu.VMEM((D, F), bf16),
            pltpu.VMEM((F, D), bf16),
            pltpu.VMEM((2, RC, 128), f32),
            pltpu.SemaphoreType.DMA((NB,)),
            pltpu.SemaphoreType.DMA((5,)),
            pltpu.SemaphoreType.DMA((NB,)),
        ],
        compiler_params=pltpu.CompilerParams(vmem_limit_bytes=100 * 1024 * 1024),
        name="kern",
    )(A_x.reshape(S, D), A_wqkv, A_wo, B_w_r.reshape(1, D), B_w_gate, B_w_up, B_w_down)
    return out.reshape(1, S, D)
```

```python
import functools
import numpy as np
import jax
import jax.numpy as jnp
from jax import lax
from jax.experimental import pallas as pl
from jax.experimental.pallas import tpu as pltpu

S, D, F = 2048, 1024, 3584
H, DH, W = 32, 32, 256
R = 256
NB = S // R
G = D // 128
RC = R // G
US = 4
NZ = 32
KB = 32
MS = 256
MERGE = 1
f32, bf16, u32 = jnp.float32, jnp.bfloat16, jnp.uint32
LOG2E = 1.4426950408889634
SCALE = 0.1767578125
EPS = float(np.float32(1e-5).astype(bf16))
NEG = -1e9 * LOG2E
O_P1 = "l q l q q L Q L Q Q"
O_P2 = "l q a l q s s s s s s s s p q a"
O_S = "e e o a q q s s s s s s s s p l l q a E E O A Q Q S S S S S S S S P L L Q A"
O_E1 = "e a e s s s s o s s s s p a"
O_E2 = "e o e E O E"


def rb(x):
    return x.astype(bf16).astype(f32)


def pack(x):
    return pltpu.bitcast(x.astype(bf16), u32)


def view(w):
    return pltpu.bitcast(w, bf16)


def recip(x):
    r = pl.reciprocal(x, approx=True)
    return r * (2.0 - x * r)


def layernorm(x):
    m = jnp.sum(x, axis=-1, keepdims=True) * (1.0 / D)
    mb = rb(m)
    c = x - mb
    v = jnp.sum(c * c, axis=-1, keepdims=True) * (1.0 / D) - (m - mb) * (m - mb)
    s = rb(jnp.sqrt(rb(rb(v) + EPS)))
    return rb(c) * recip(s)


def kernel(x_hbm, wqkv_hbm, wo_hbm, wr_ref, wg_hbm, wu_hbm, wd_hbm, out_hbm,
           x_buf, x1_buf, q_buf, k_buf, v_buf, o_buf, wqkv_buf, wo_buf,
           wg_buf, wu_buf, wd_buf, zero_ref, sem_x, sem_q, sem_w, sem_o):
    x_hbm, wqkv_hbm, wo_hbm, wg_hbm, wu_hbm, wd_hbm, out_hbm = (
        r.bitcast(u32) for r in (x_hbm, wqkv_hbm, wo_hbm, wg_hbm, wu_hbm, wd_hbm, out_hbm))
    HB = NB + 1
    best = pl.ds((2 * NB + 1) * R // 2, RC)

    def rows_of(b, n=R, off=0):
        return pl.ds(pl.multiple_of(b * (R // 2) + off // 2, RC // 2), n // 2)

    def x_copy(b):
        return pltpu.make_async_copy(x_hbm.at[rows_of(b)], x_buf.at[rows_of(b)], sem_x.at[b])

    def out_copy(b):
        return pltpu.make_async_copy(x_buf.at[rows_of(b)], out_hbm.at[rows_of(b)], sem_o.at[b])

    def cols_of(g, n=128):
        return pl.ds(pl.multiple_of(g * n, n), n)

    def wqkv_copies(j):
        return [pltpu.make_async_copy(wqkv_hbm.at[:, cols_of(j + t * (G // 2), 256)],
                                      wqkv_buf.at[:, cols_of(j + t * (G // 2), 256)], sem_q.at[j])
                for t in range(3)]

    w_copies = [
        pltpu.make_async_copy(wo_hbm, wo_buf, sem_w.at[0]),
        pltpu.make_async_copy(wg_hbm, wg_buf, sem_w.at[1]),
        pltpu.make_async_copy(wu_hbm, wu_buf, sem_w.at[2]),
        pltpu.make_async_copy(wd_hbm, wd_buf, sem_w.at[3]),
    ]
    x_copy(0).start()
    for c in wqkv_copies(0):
        c.start()
    x_copy(1).start()

    for i in range(NZ):
        zero_ref[i] = 0
    zc = [0]

    def opaque_zero():
        zc[0] = (zc[0] + 1) % NZ
        return zero_ref[zc[0]]

    lane = lax.broadcasted_iota(jnp.int32, (KB, 128), 1)
    row = lax.broadcasted_iota(jnp.int32, (KB, 128), 0)

    def ln_stage(b, g):
        h = layernorm(view(x_buf[rows_of(b, RC, g * RC), :]).astype(f32))
        yield
        x_buf[rows_of(b + HB, RC, g * RC), :] = pack(h)

    def dense(lhs_ref, b, w_ref, c):
        for m in range(0, R, MS):
            z = opaque_zero()
            yield jnp.dot(view(lhs_ref[rows_of(b + z, MS, m), :]), view(w_ref[:, cols_of(c + z)]),
                          preferred_element_type=f32)

    def qkv_stage(b, g):
        for t, (dst, mul) in enumerate(((q_buf, SCALE * LOG2E), (k_buf, None), (v_buf, None))):
            for i, y in enumerate(dense(x_buf, b + HB, wqkv_buf, g + t * G)):
                dst[g, rows_of(b, MS, i * MS), :] = pack(y if mul is None else y * mul)
                yield

    def blockdiag(w):
        ln = lane[: KB // 2] // DH
        z = jnp.zeros_like(w)
        return pltpu.bitcast(jnp.concatenate([jnp.where(ln == hh, w, z) for hh in range(4)], axis=0), bf16)

    def segment(x, op, fill):
        ln = lane[: x.shape[0]] // DH
        out = None
        for hh in range(4):
            r = op(jnp.where(ln == hh, x, fill), axis=-1, keepdims=True)
            out = r if out is None else jnp.where(ln == hh, r, out)
        return out

    def att_stage(b, g, first):
        nt = R // KB
        us = list(range(nt if first else 0, 2 * nt))
        lo = {u: max(0, u - nt) for u in us}
        hi = {u: min(nt, u + 1) for u in us}
        causal = lane % KB <= row
        s = {}
        for u in us:
            kt = k_buf[g, rows_of(b, KB, (u - nt) * KB), :]
            qu = view(q_buf[g, rows_of(b, (hi[u] - lo[u]) * KB, lo[u] * KB), :])
            su = lax.dot_general(qu, blockdiag(kt), (((1,), (1,)), ((), ())), preferred_element_type=f32)
            for i in range(lo[u], hi[u]):
                s[u, i] = su[(i - lo[u]) * KB: (i - lo[u] + 1) * KB]
            if u >= nt:
                i = u - nt
                if first:
                    s[u, i] = jnp.where(causal, s[u, i], NEG)
                elif MERGE:
                    s[u, i] = jnp.where(causal, s[u, i], s.pop((i, i)))
                else:
                    s[u, i] = jnp.where(causal, s[u, i], NEG)
                    s[i, i] = jnp.where(causal, NEG, s[i, i])
        yield
        p = {}
        linv = {}
        for i in range(nt):
            mine = [u for u in us if (u, i) in s]
            m = functools.reduce(jnp.maximum, [s[u, i] for u in mine])
            m = segment(m, jnp.max, -np.inf)
            e = [jnp.exp2(s[u, i] - m) for u in mine]
            linv[i] = recip(segment(functools.reduce(jnp.add, e), jnp.sum, 0.0))
            for u, eu in zip(mine, e):
                if MERGE and not first and u == i + nt:
                    p[u, i] = jnp.where(causal, eu, 0.0).astype(bf16)
                    p[i, i] = jnp.where(causal, 0.0, eu).astype(bf16)
                else:
                    p[u, i] = eu.astype(bf16)
            yield
        acc = {}
        for u in us:
            vt = v_buf[g, rows_of(b, KB, (u - nt) * KB), :]
            pu = jnp.concatenate([p[u, i] for i in range(lo[u], hi[u])], axis=0)
            ou = jnp.dot(pu, blockdiag(vt), preferred_element_type=f32)
            for i in range(lo[u], hi[u]):
                t = ou[(i - lo[u]) * KB: (i - lo[u] + 1) * KB]
                acc[i] = t if i not in acc else acc[i] + t
        o = pack(jnp.concatenate([acc[i] * linv[i] for i in range(nt)], axis=0))
        yield
        o_buf[rows_of(b), cols_of(g)] = o

    def out_stage(b, g):
        for i, a in enumerate(dense(o_buf, b, wo_buf, g)):
            rr = rows_of(b, MS, i * MS)
            x1_buf[rr, cols_of(g)] = pack(view(x_buf[rr, cols_of(g)]).astype(f32) + rb(a))
            yield

    def router(h1):
        return rb(jnp.sum(h1 * wr_ref[...].astype(f32), axis=-1, keepdims=True))

    def get_best():
        return pltpu.bitcast(x_buf[best, 0:128], f32), pltpu.bitcast(x_buf[best, 128:256], f32)

    def set_best(v, i):
        x_buf[best, 0:128] = pltpu.bitcast(v, u32)
        x_buf[best, 128:256] = pltpu.bitcast(i, u32)

    def epi_stage(b, g, valid=None):
        src = b if valid is None else jnp.maximum(b, 0)
        dst = b if valid is None else jnp.where(valid, b, NB)
        x1 = view(x1_buf[rows_of(src, RC, g * RC), :]).astype(f32)
        yield
        h1 = rb(layernorm(x1))
        x_buf[rows_of(dst, RC, g * RC), :] = pack(x1 + h1)
        r = jnp.broadcast_to(router(h1), (RC, 128))
        if valid is not None:
            r = jnp.where(valid, r, -np.inf)
        bv, bi = get_best()
        gt = r > bv
        set_best(jnp.where(gt, r, bv), jnp.where(gt, (row + (b * R + g * RC)).astype(f32), bi))

    def steps(order, pre=None, unroll=1, **stages):
        order = [t[0] for t in order.split() for _ in range(R // MS if t in "qoQO" else 1)]
        n = 2 if any(t.isupper() for t in order) else 1
        alias = {"s": "a", "p": "a"}

        def body(j, _):
            if pre is not None:
                pre(j)
            live = {}
            for t in order:
                name = alias.get(t.lower(), t.lower())
                key = (name, t.isupper())
                if key not in live:
                    live[key] = stages[name](j * n + int(t.isupper()))
                next(live[key], None)
            assert len(live) == n * len(stages)
            for gen in live.values():
                assert next(gen, 1) == 1
        lax.fori_loop(0, G // n, body, None, unroll=unroll)

    def unrolled(stage):
        gens = [stage(g) for g in range(G)]
        while gens:
            gens = [gen for gen in gens if next(gen, 1) is None]

    P = functools.partial

    x_copy(0).wait()
    unrolled(P(ln_stage, 0))

    def layer(li, _):
        set_best(jnp.full((RC, 128), -np.inf, f32), jnp.zeros((RC, 128), f32))

        def first_layer(fn):
            pl.when(li == 0)(fn)

        def send(b):
            @pl.when(li == 1)
            def _():
                out_copy(b).start()

        def stream_wqkv(j):
            @first_layer
            def _():
                @pl.when(j + 1 < G // 2)
                def _():
                    for c in wqkv_copies(j + 1):
                        c.start()

                @pl.when(j + 1 == G // 2)
                def _():
                    x_copy(2).start()
                    x_copy(3).start()
                    w_copies[0].start()
                for c in wqkv_copies(j):
                    c.wait()

        first_layer(lambda: x_copy(1).wait())
        steps(O_P1, pre=stream_wqkv, q=P(qkv_stage, 0), l=P(ln_stage, 1))

        @first_layer
        def _():
            x_copy(2).wait()
            for b in range(4, NB):
                x_copy(b).start()
        steps(O_P2, a=P(att_stage, 0, first=True), q=P(qkv_stage, 1), l=P(ln_stage, 2))

        @first_layer
        def _():
            w_copies[0].wait()
            for c in w_copies[1:]:
                c.start()

        def steady(b, _):
            @first_layer
            def _():
                pl.when(b + 2 < NB)(lambda: x_copy(b + 2).wait())
            steps(O_S, unroll=US, e=P(epi_stage, b - 2, valid=b >= 2), o=P(out_stage, b - 1),
                  a=P(att_stage, b, first=False), q=P(qkv_stage, b + 1),
                  l=P(ln_stage, jnp.where(b + 2 < NB, b + 2, 0)))
            pl.when(b >= 2)(lambda: send(b - 2))
        lax.fori_loop(1, NB - 1, steady, None)
        b = NB - 1
        steps(O_E1, e=P(epi_stage, b - 2), o=P(out_stage, b - 1), a=P(att_stage, b, first=False))
        send(b - 2)
        steps(O_E2, e=P(epi_stage, NB - 2), o=P(out_stage, NB - 1))
        send(NB - 2)
        unrolled(P(epi_stage, NB - 1))
        send(NB - 1)

        bv, bi = get_best()
        idx = jnp.min(jnp.where(bv == jnp.max(bv), bi, float(S - 1))).astype(jnp.int32)
        t0 = (idx // 16) * 16
        tt = pl.ds(pl.multiple_of(t0 // 2, 8), 8)

        @first_layer
        def _():
            for c in w_copies[1:]:
                c.wait()
        x1 = view(x1_buf[tt, :]).astype(f32)
        h1 = rb(layernorm(x1))
        hb = h1.astype(bf16)
        FC = 512
        y = None
        for c in range(0, F, FC):
            gt = rb(jnp.dot(hb, view(wg_buf[:, c:c + FC]), preferred_element_type=f32))
            gt = rb(gt * jax.nn.sigmoid(gt))
            up = rb(jnp.dot(hb, view(wu_buf[:, c:c + FC]), preferred_element_type=f32))
            if c == 0:
                acts = []
            acts.append((gt * up).astype(bf16))
        for i, c in enumerate(range(0, F, FC)):
            yc = jnp.dot(acts[i], view(wd_buf[c // 2:(c + FC) // 2, :]), preferred_element_type=f32)
            y = yc if y is None else y + yc
        y = rb(rb(y) * rb(jax.nn.sigmoid(router(h1))))
        sel = lax.broadcasted_iota(jnp.int32, (16, D), 0) == idx - t0
        new = rb(x1 + jnp.where(sel, rb(h1 + y), h1))

        @pl.when(li == 1)
        def _():
            for b in range(NB):
                out_copy(b).wait()
        x_buf[tt, :] = pack(new)

        @first_layer
        def _():
            x_buf[pl.ds(pl.multiple_of(t0 // 2 + HB * R // 2, 8), 8), :] = pack(layernorm(new))

        @pl.when(li == 1)
        def _():
            c = pltpu.make_async_copy(x_buf.at[tt], out_hbm.at[tt], sem_o.at[0])
            c.start()
            c.wait()

    lax.fori_loop(0, 2, layer, None)


@jax.jit
def pallas_interleave_layers__sliding_block__moe_arch_mod__prompt_kernel(
    A_x, A_wqkv, A_wo, B_x, B_w_r, B_w_gate, B_w_up, B_w_down,
):
    any_spec = pl.BlockSpec(memory_space=pl.ANY)
    out = pl.pallas_call(
        kernel,
        out_shape=jax.ShapeDtypeStruct((S, D), bf16),
        in_specs=[any_spec, any_spec, any_spec, pl.BlockSpec(memory_space=pltpu.VMEM),
                  any_spec, any_spec, any_spec],
        out_specs=any_spec,
        scratch_shapes=[
            pltpu.VMEM(((2 * S + R) // 2 + RC, D), u32),
            pltpu.VMEM((S // 2, D), u32),
            pltpu.VMEM((G, S // 2, 128), u32),
            pltpu.VMEM((G, S // 2, 128), u32),
            pltpu.VMEM((G, S // 2, 128), u32),
            pltpu.VMEM((S // 2, D), u32),
            pltpu.VMEM((D // 2, 3 * D), u32),
            pltpu.VMEM((D // 2, D), u32),
            pltpu.VMEM((D // 2, F), u32),
            pltpu.VMEM((D // 2, F), u32),
            pltpu.VMEM((F // 2, D), u32),
            pltpu.SMEM((NZ,), jnp.int32),
            pltpu.SemaphoreType.DMA((NB,)),
            pltpu.SemaphoreType.DMA((G // 2,)),
            pltpu.SemaphoreType.DMA((4,)),
            pltpu.SemaphoreType.DMA((NB,)),
        ],
        compiler_params=pltpu.CompilerParams(vmem_limit_bytes=100 * 1024 * 1024, flags={"XLA_TPU_FORCE_LP_LLO_SCHEDULER": True}),
        name="kern",
    )(A_x.reshape(S, D), A_wqkv, A_wo, B_w_r.reshape(1, D), B_w_gate, B_w_up, B_w_down)
    return out.reshape(1, S, D)
```

```python
import functools
import numpy as np
import jax
import jax.numpy as jnp
from jax import lax
from jax.experimental import pallas as pl
from jax.experimental.pallas import tpu as pltpu

S, D, F = 2048, 1024, 3584
DH = 32
R = 256
NB = S // R
G = D // 128
RC = R // G
KB = 32
NT = R // KB
HB = NB + 1
f32, bf16, u32 = jnp.float32, jnp.bfloat16, jnp.uint32
LOG2E = 1.4426950408889634
SCALE = float(np.float32(DH ** -0.5).astype(bf16))
EPS = float(np.float32(1e-5).astype(bf16))
NEG = -1e9 * LOG2E
ALL = range(G)

AQ = 4
ER = 32
LR = 32
NZ = 6
XM = 1
O_P1 = "l q q q"
O_P2 = "q l a q p p q a"
O_S = "e o l a q p q p q a"
O_E1 = "e a o p p a"
U_P2 = 2
U_E1 = 2
O_E2 = "o1 e e o1 e e o1 e e o1 e e o1 e e o1 e e o1 e o1 e e e"
FPLAN = "G2 G1 V1 G1 D0 V1 G1 D0 V1 G1 D0 V1 G1 D0 V1 G1 D0 V1 G1 D0 V1 G1 D0 V1 G1 D0 V1 G1 D0 V1 G1 D0 V1 G1 D0 V1 D0 V1 D0 V1"


def rb(x):
    return x.astype(bf16).astype(f32)


def recip(x):
    r = pl.reciprocal(x, approx=True)
    return r * (2.0 - x * r)


def layernorm(x):
    m = jnp.sum(x, axis=-1, keepdims=True) * (1.0 / D)
    mb = rb(m)
    c = x - mb
    v = jnp.sum(c * c, axis=-1, keepdims=True) * (1.0 / D) - (m - mb) * (m - mb)
    s = rb(jnp.sqrt(rb(rb(v) + EPS)))
    return rb(c) * recip(s)


def aligned(i, n):
    return pl.ds(i * n if isinstance(i, int) else pl.multiple_of(i * n, n), n)


def window(ref, rows, div):
    blk, span, off, n = rows
    return ref.at[:, aligned(blk, span // div)], pl.ds(off // div, n // div)


def put(ref, rows, cols, x):
    ref, rows = window(ref, rows, 1)
    for i, c in enumerate(cols if isinstance(cols, range) else [cols]):
        ref[c, rows, :] = x[:, i * 128:(i + 1) * 128].astype(bf16)


def words(ref, rows, cols):
    ref, rows = window(ref.bitcast(u32), rows, 2)
    return jnp.concatenate([ref[c, rows, :] for c in (cols if isinstance(cols, range) else [cols])], axis=1)


def get(ref, rows, cols):
    return pltpu.bitcast(words(ref, rows, cols), bf16)


def rows_of(b, n=R, off=0):
    return (b - 1, R, off + R, n) if off < 0 else (b, R, off, n)


def chunk_of(b, g, n=RC, off=0):
    return (b, R, g * RC + off, n) if isinstance(g, int) else (b * G + g, RC, off, n)


def start(copies):
    for c in copies:
        c.start()


def wait(copies):
    for c in copies:
        c.wait()


def run(gen):
    for _ in gen:
        pass


def kernel(x_hbm, wqkv_hbm, wo_hbm, wr_ref, wg_hbm, wu_hbm, wd_hbm, out_hbm,
           x_buf, x1_buf, q_buf, k_buf, v_buf, o_buf, s_buf, wqkv_buf, wo_buf,
           wg_buf, wu_buf, wd_buf, wr_buf, xcol_buf, zero_ref, sem_x, sem_q, sem_w, sem_o):
    def x_copy(b):
        return [pltpu.make_async_copy(x_hbm.at[aligned(b, R), aligned(c, 128)], x_buf.at[c, aligned(b, R)],
                                      sem_x.at[b]) for c in ALL]

    def out_copy(b, n, sem):
        return [pltpu.make_async_copy(x_buf.at[c, aligned(b, n)], out_hbm.at[aligned(b, n), aligned(c, 128)],
                                      sem_o.at[sem]) for c in ALL]

    def w_copy(src, dst, cols, sem):
        return [pltpu.make_async_copy(src.at[:, aligned(c, 128)], dst.at[c], sem) for c in cols]

    def wqkv_copy(g):
        return w_copy(wqkv_hbm, wqkv_buf, range(g, 3 * G, G), sem_q.at[g])

    wo_copy = w_copy(wo_hbm, wo_buf, ALL, sem_w.at[0])
    ffn_copy = (w_copy(wg_hbm, wg_buf, range(F // 128), sem_w.at[1])
                + w_copy(wu_hbm, wu_buf, range(F // 128), sem_w.at[1])
                + w_copy(wd_hbm, wd_buf, ALL, sem_w.at[1]))
    start(x_copy(0))
    start(wqkv_copy(0))

    for i in range(NZ):
        zero_ref[i] = 0
    zeros = [zero_ref[i] for i in range(NZ)]
    count = {"z": 0, "s": 0}

    def opaque_zero():
        count["z"] += 1
        return zeros[count["z"] % NZ]

    lane = lax.broadcasted_iota(jnp.int32, (KB, 128), 1)
    row = lax.broadcasted_iota(jnp.int32, (KB, 128), 0)
    head = lax.broadcasted_iota(jnp.int32, (1, 128), 1) // DH
    wr_buf[...] = jnp.broadcast_to(wr_ref[...].astype(f32).reshape(1, D), (8, D))
    full = (0, D, 0, D)

    def ln_stage(b, g):
        for r in range(0, RC, LR):
            h = layernorm(get(x_buf, chunk_of(b, g, LR, r), ALL).astype(f32))
            put(x_buf, chunk_of(b + HB, g, LR, r), ALL, h)
            yield

    def qkv_stage(b, g):
        for t, dst in enumerate((q_buf, k_buf, v_buf)):
            y = jnp.dot(get(x_buf, rows_of(b + HB + opaque_zero()), ALL), get(wqkv_buf, full, g + t * G),
                        preferred_element_type=f32)
            put(dst, rows_of(b), g, y if t else y * (SCALE * LOG2E))
            yield

    def blockdiag(w):
        z = jnp.zeros_like(w)
        return pltpu.bitcast(jnp.concatenate([jnp.where(head == h, w, z) for h in range(4)], axis=0), bf16)

    def segment(x, op, fill):
        out = None
        for h in range(4):
            r = op(jnp.where(head == h, x, fill), axis=-1, keepdims=True)
            out = r if out is None else jnp.where(head == h, r, out)
        return out

    def att_stage(b, g, first=False):
        count["s"] ^= 1
        s_put, s_get = s_buf.at[count["s"]], s_buf.at[count["s"] + zeros[0]]
        causal = lane % KB <= row
        parts = []
        for i0 in range(0, NT, AQ):
            tiles = {u: range(max(i0, u - NT), min(i0 + AQ, u + 1))
                     for u in range(NT if first else i0, NT + i0 + AQ)}
            bz = b + zeros[i0 // AQ] if i0 else b
            s = {}
            for u, qs in tiles.items():
                su = lax.dot_general(get(q_buf, rows_of(b, len(qs) * KB, qs[0] * KB), g),
                                     blockdiag(words(k_buf, rows_of(bz, KB, (u - NT) * KB), g)),
                                     (((1,), (1,)), ((), ())), preferred_element_type=f32)
                for n, i in enumerate(qs):
                    s[u, i] = su[n * KB:(n + 1) * KB]
                if u - NT >= i0:
                    i = u - NT
                    s[u, i] = jnp.where(causal, s[u, i], NEG if first else s.pop((i, i)))
            m = {}
            for (u, i), t in s.items():
                s_put[u, i * KB:(i + 1) * KB, :] = t
                m[i] = jnp.maximum(m[i], t) if i in m else t
            parts.append((tiles, bz, {i: segment(t, jnp.max, -np.inf) for i, t in m.items()}))
        yield
        outs = []
        for tiles, bz, m in parts:
            diag, l, acc = {}, {}, {}

            def prob(u, i):
                if i in diag and u == i + NT:
                    return diag[i]
                e = jnp.exp2(s_get[u + NT if u == i else u, i * KB:(i + 1) * KB, :] - m[i])
                l[i] = l[i] + e if i in l else e
                if u != i:
                    return e
                diag[i] = jnp.where(causal, e, 0.0)
                return jnp.where(causal, 0.0, e)

            for u, qs in tiles.items():
                pu = jnp.concatenate([prob(u, i) for i in qs], axis=0).astype(bf16)
                ou = jnp.dot(pu, blockdiag(words(v_buf, rows_of(bz, KB, (u - NT) * KB), g)),
                             preferred_element_type=f32)
                for n, i in enumerate(qs):
                    t = ou[n * KB:(n + 1) * KB]
                    acc[i] = acc[i] + t if i in acc else t
            outs += [acc[i] * recip(segment(l[i], jnp.sum, 0.0)) for i in sorted(acc)]
            yield
        put(o_buf, rows_of(b), g, jnp.concatenate(outs, axis=0))

    def out_proj(b, n, off, cols):
        z = opaque_zero()
        a = jnp.dot(get(o_buf, rows_of(b + z, n, off), ALL),
                    get(wo_buf, (z, D, 0, D) if n < R else full, cols), preferred_element_type=f32)
        put(x1_buf, rows_of(b, n, off), cols, get(x_buf, rows_of(b + z, n, off), cols).astype(f32) + rb(a))

    def out_stage(b, g):
        out_proj(b, R, 0, g)
        yield

    def router(h):
        wr = jnp.concatenate([wr_buf[...]] * (h.shape[0] // 8), axis=0)
        return rb(jnp.sum(h * wr, axis=-1, keepdims=True))

    best = x_buf.bitcast(u32).at[:, pl.ds((HB + NB) * R // 2, ER)]

    def epi_stage(b, g, valid=None):
        src = b if valid is None else jnp.maximum(b, 0)
        dst = b if valid is None else jnp.where(valid, b, NB)
        for r0 in range(0, RC, ER):
            x1 = get(x1_buf, chunk_of(src, g, ER, r0), ALL).astype(f32)
            h1 = layernorm(x1)
            put(x1_buf, chunk_of(dst + HB, g, ER, r0), ALL, h1)
            h1 = rb(h1)
            put(x_buf, chunk_of(dst, g, ER, r0), ALL, x1 + h1)
            r = jnp.broadcast_to(router(h1), (ER, 128))
            if valid is not None:
                r = jnp.where(valid, r, -np.inf)
            bv = pltpu.bitcast(best[0], f32)
            best[0] = pltpu.bitcast(jnp.where(r > bv, r, bv), u32)
            best[1] = jnp.where(r > bv, pltpu.bitcast(row[:ER] + (b * R + g * RC + r0), u32), best[1])
            yield

    def ffn(xs):
        xs = jnp.broadcast_to(xs, (8, D))
        if XM:
            eye = lax.broadcasted_iota(jnp.int32, (128, 128), 0) == lax.broadcasted_iota(jnp.int32, (128, 128), 1)
            for c in range(0, D, 128):
                d = jnp.where(eye, jnp.concatenate([xs[:, c:c + 128]] * 16, axis=0), 0.0).astype(bf16)
                xcol_buf[c:c + 128, :] = jnp.dot(d, jnp.ones((128, 128), bf16), preferred_element_type=f32)
        else:
            for c in range(0, D, 128):
                xcol_buf[c:c + 128, :] = jnp.concatenate([xs[:, c:c + 128]] * 16, axis=0).T
        hb = xs.astype(bf16)

        def on_mxu(cols):
            return [jnp.dot(hb, get(w, full, cols), preferred_element_type=f32) for w in (wg_buf, wu_buf)]

        def on_vpu(cols):
            xcol = xcol_buf.at[pl.ds(pl.multiple_of(opaque_zero() * cols[0], 16), D)]
            acc = [0.0, 0.0]
            for k in range(0, D, 16):
                xk = jnp.concatenate([xcol[k:k + 16, :]] * len(cols), axis=1)
                for t, w in enumerate((wg_buf, wu_buf)):
                    prod = get(w, (0, D, k, 16), cols).astype(f32) * xk
                    acc[t] = (acc[t] + prod[:8]) + prod[8:]
            return [jnp.broadcast_to(jnp.sum(a, axis=0, keepdims=True), a.shape) for a in acc]

        def act(gate, up):
            gate = rb(gate)
            return (rb(gate * jax.nn.sigmoid(gate)) * rb(up)).astype(bf16)

        queue, c, y = [], 0, 0.0
        for t in FPLAN.split():
            cols = range(c, c + int(t[1:]))
            c += len(cols)
            if t[0] == "G":
                queue.append((cols, act(*on_mxu(cols))))
                continue
            cols, a = queue.pop(0) if t[0] == "D" else (cols, act(*on_vpu(cols)))
            y = y + jnp.dot(a, get(wd_buf, (0, F, cols[0] * 128, len(cols) * 128), ALL),
                            preferred_element_type=f32)
        assert c * 128 == F and not queue
        return rb(rb(y) * rb(jax.nn.sigmoid(router(xs))))

    def steps(name, order, unroll=G, pre=None, **stages):
        order = order.split()
        pair = 1 + any(t.isupper() for t in order)

        def body(j, _):
            for n in range(0, unroll, pair):
                if pre is not None:
                    pre(j * unroll + n)
                live = {}
                for t in order:
                    key = (t.lower().replace("p", "a"), int(t.isupper()))
                    if key not in live:
                        live[key] = stages[key[0]](j * unroll + n + key[1])
                    next(live[key], None)
                assert all(next(gen, 1) == 1 for gen in live.values())
        if unroll == G:
            body(0, None)
        else:
            lax.fori_loop(0, G // unroll, body, None)

    P = functools.partial

    def stream_weights(g):
        if g + 2 < G:
            start(wqkv_copy(g + 2))
        elif g + 2 == G:
            start(x_copy(2) + wo_copy)
        wait(wqkv_copy(g))
        if g == 0:
            wait(x_copy(1))

    wait(x_copy(0))
    start(x_copy(1))
    start(wqkv_copy(1))
    for g in ALL:
        run(ln_stage(0, g))
    steps("P1", O_P1, pre=stream_weights, q=P(qkv_stage, 0), l=P(ln_stage, 1))
    wait(x_copy(2))
    for b in range(3, NB):
        start(x_copy(b))

    def layer(li, _):
        best[0] = pltpu.bitcast(jnp.full((ER, 128), -np.inf, f32), u32)
        best[1] = jnp.zeros((ER, 128), u32)
        steps("P2", O_P2, U_P2, a=P(att_stage, 0, first=True), q=P(qkv_stage, 1), l=P(ln_stage, 2))

        @pl.when(li == 0)
        def _():
            wait(wo_copy)
            for b in range(3, NB):
                wait(x_copy(b))
            start(ffn_copy)

        def steady(b, _):
            steps("S", O_S, e=P(epi_stage, b - 2, valid=b >= 2), o=P(out_stage, b - 1), a=P(att_stage, b),
                  q=P(qkv_stage, (b + 1) & (NB - 1)), l=P(ln_stage, (b + 2) & (NB - 1)))
        lax.fori_loop(1, NB - li, steady, None)

        @pl.when(li == 1)
        def _():
            start(out_copy(0, (NB - 3) * R, 0))
            steps("E1", O_E1, U_E1, e=P(epi_stage, NB - 3), o=P(out_stage, NB - 2), a=P(att_stage, NB - 1))
            start(out_copy(NB - 3, R, 1))

        n_out = n_epi = 0
        for t in O_E2.split():
            if t == "e":
                run(epi_stage(NB - 2 + n_epi // G, n_epi % G))
                n_epi += 1
            else:
                out_proj(NB - 1, int(t[1:]) * RC, n_out * RC, ALL)
                n_out += int(t[1:])
        assert (n_out, n_epi) == (G, 2 * G)

        pl.when(li == 0)(lambda: wait(ffn_copy))
        pl.when(li == 1)(lambda: start(out_copy(NB // 2 - 1, 2 * R, 2)))

        bv, bi = pltpu.bitcast(best[0], f32), pltpu.bitcast(best[1], jnp.int32).astype(f32)
        idx = jnp.min(jnp.where(bv == jnp.max(bv, axis=0, keepdims=True), bi, float(S - 1))).astype(jnp.int32)
        tile = lax.shift_right_logical(idx, 4)
        x1 = get(x1_buf, (tile, 16, 0, 16), ALL).astype(f32)
        h1 = get(x1_buf, (tile + HB * R // 16, 16, 0, 16), ALL).astype(f32)
        sel = lax.broadcasted_iota(jnp.int32, (16, D), 0) == idx - tile * 16
        y = ffn(jnp.sum(jnp.where(sel, h1, 0.0), axis=0, keepdims=True))
        new = rb(x1 + jnp.where(sel, rb(h1 + jnp.concatenate([y, y], axis=0)), h1))

        @pl.when(li == 0)
        def _():
            put(x_buf, (tile, 16, 0, 16), ALL, new)
            h = layernorm(new)
            put(x_buf, (tile + HB * R // 16, 16, 0, 16), ALL, h)

            @pl.when(idx < R)
            def _():
                for t, dst in enumerate((q_buf, k_buf, v_buf)):
                    y = jnp.dot(h.astype(bf16), get(wqkv_buf, full, range(t * G, (t + 1) * G)),
                                preferred_element_type=f32)
                    put(dst, (tile, 16, 0, 16), ALL, y if t else y * (SCALE * LOG2E))

        @pl.when(li == 1)
        def _():
            wait(out_copy(0, (NB - 3) * R, 0) + out_copy(NB - 3, R, 1) + out_copy(NB // 2 - 1, 2 * R, 2))
            put(x_buf, (tile, 16, 0, 16), ALL, new)
            start(out_copy(tile, 16, 0))
            wait(out_copy(tile, 16, 0))

    lax.fori_loop(0, 2, layer, None)


@jax.jit
def pallas_interleave_layers__sliding_block__moe_arch_mod__prompt_kernel(
    A_x, A_wqkv, A_wo, B_x, B_w_r, B_w_gate, B_w_up, B_w_down,
):
    any_spec = pl.BlockSpec(memory_space=pl.ANY)

    def tiled(rows, cols):
        return pltpu.VMEM((cols // 128, rows, 128), bf16)

    out = pl.pallas_call(
        kernel,
        out_shape=jax.ShapeDtypeStruct((S, D), bf16),
        in_specs=[any_spec, any_spec, any_spec, pl.BlockSpec(memory_space=pltpu.VMEM),
                  any_spec, any_spec, any_spec],
        out_specs=any_spec,
        scratch_shapes=[
            tiled((HB + NB) * R + 2 * RC, D),
            tiled(2 * HB * R, D),
            tiled(S, D), tiled(S, D), tiled(S, D), tiled(S, D),
            pltpu.VMEM((2, 2 * NT, R, 128), f32),
            tiled(D, 3 * D), tiled(D, D), tiled(D, F), tiled(D, F), tiled(F, D),
            pltpu.VMEM((8, D), f32),
            pltpu.VMEM((D, 128), f32),
            pltpu.SMEM((NZ,), jnp.int32),
            pltpu.SemaphoreType.DMA((NB,)),
            pltpu.SemaphoreType.DMA((G,)),
            pltpu.SemaphoreType.DMA((2,)),
            pltpu.SemaphoreType.DMA((3,)),
        ],
        compiler_params=pltpu.CompilerParams(
            vmem_limit_bytes=100 * 1024 * 1024, disable_bounds_checks=True,
            flags={"XLA_TPU_FORCE_LP_LLO_SCHEDULER": True}),
        name="kern",
    )(A_x.reshape(S, D), A_wqkv, A_wo, B_w_r, B_w_gate, B_w_up, B_w_down)
    return out.reshape(1, S, D)
```

```python
import functools
import numpy as np
import jax
import jax.numpy as jnp
from jax import lax
from jax.experimental import pallas as pl
from jax.experimental.pallas import tpu as pltpu

S, D, F = 2048, 1024, 3584
DH = 32
R = 256
NB = S // R
G = D // 128
RC = R // G
KB = 32
NT = R // KB
HB = NB + 1
f32, bf16, u32 = jnp.float32, jnp.bfloat16, jnp.uint32
LOG2E = 1.4426950408889634
SCALE = float(np.float32(DH ** -0.5).astype(bf16))
EPS = float(np.float32(1e-5).astype(bf16))
NEG = -1e9 * LOG2E
ALL = range(G)

AQ = 4
ER = 16
LR = 16
NZ = 6
XM = 0
O_P1 = "q l q l q"
O_P2 = "q l a q l p p q a"
O_S = "l o l a q e p q e p q a"
O_E1 = "e a o e p p a"
U_P1 = 2
U_P2 = 2
U_E1 = 2
O_E2 = "o1 e4 o1 e4 o1 e4 o1 e4 o1 e4 o1 e4 o1 e2 o1"
FPLAN = "G2 G1 V1 G1 D0 V1 G1 D0 V1 G1 D0 V1 G1 D0 V1 G1 D0 V1 G1 D0 V1 G1 D0 V1 G1 D0 V1 G1 D0 V1 G1 D0 V1 G1 D0 V1 D0 V1 D0 V1"


def rb(x):
    return x.astype(bf16).astype(f32)


def recip(x):
    r = pl.reciprocal(x, approx=True)
    return r * (2.0 - x * r)


def layernorm(x):
    m = jnp.sum(x, axis=-1, keepdims=True) * (1.0 / D)
    mb = rb(m)
    c = x - mb
    v = jnp.sum(c * c, axis=-1, keepdims=True) * (1.0 / D) - (m - mb) * (m - mb)
    s = rb(jnp.sqrt(rb(rb(v) + EPS)))
    return rb(c) * recip(s)


def aligned(i, n):
    return pl.ds(i * n if isinstance(i, int) else pl.multiple_of(i * n, n), n)


def window(ref, rows, div):
    blk, span, off, n = rows
    return ref.at[:, aligned(blk, span // div)], pl.ds(off // div, n // div)


def put(ref, rows, cols, x):
    ref, rows = window(ref, rows, 1)
    for i, c in enumerate(cols if isinstance(cols, range) else [cols]):
        ref[c, rows, :] = x[:, i * 128:(i + 1) * 128].astype(bf16)


def words(ref, rows, cols):
    ref, rows = window(ref.bitcast(u32), rows, 2)
    return jnp.concatenate([ref[c, rows, :] for c in (cols if isinstance(cols, range) else [cols])], axis=1)


def get(ref, rows, cols):
    return pltpu.bitcast(words(ref, rows, cols), bf16)


def rows_of(b, n=R, off=0):
    return (b - 1, R, off + R, n) if off < 0 else (b, R, off, n)


def chunk_of(b, g, n=RC, off=0):
    return (b, R, g * RC + off, n) if isinstance(g, int) else (b * G + g, RC, off, n)


def start(copies):
    for c in copies:
        c.start()


def wait(copies):
    for c in copies:
        c.wait()


def run(gen):
    for _ in gen:
        pass


def kernel(x_hbm, wqkv_hbm, wo_hbm, wr_ref, wg_hbm, wu_hbm, wd_hbm, out_hbm,
           x_buf, x1_buf, q_buf, k_buf, v_buf, o_buf, s_buf, wqkv_buf, wo_buf,
           wg_buf, wu_buf, wd_buf, wr_buf, xcol_buf, zero_ref, sem_x, sem_q, sem_w, sem_o):
    def x_copy(b):
        return [pltpu.make_async_copy(x_hbm.at[aligned(b, R), aligned(c, 128)], x_buf.at[c, aligned(b, R)],
                                      sem_x.at[b]) for c in ALL]

    def out_copy(b, n, sem):
        return [pltpu.make_async_copy(x_buf.at[c, aligned(b, n)], out_hbm.at[aligned(b, n), aligned(c, 128)],
                                      sem_o.at[sem]) for c in ALL]

    def w_copy(src, dst, cols, sem):
        return [pltpu.make_async_copy(src.at[:, aligned(c, 128)], dst.at[c], sem) for c in cols]

    def wqkv_copy(j):
        return w_copy(wqkv_hbm, wqkv_buf, [j * U_P1 + n + t * G for n in range(U_P1) for t in range(3)], sem_q.at[j])

    wo_copy = w_copy(wo_hbm, wo_buf, ALL, sem_w.at[0])
    ffn_copy = (w_copy(wg_hbm, wg_buf, range(F // 128), sem_w.at[1])
                + w_copy(wu_hbm, wu_buf, range(F // 128), sem_w.at[1])
                + w_copy(wd_hbm, wd_buf, ALL, sem_w.at[1]))
    start(x_copy(0))
    start(wqkv_copy(0))

    for i in range(NZ):
        zero_ref[i] = 0
    zeros = [zero_ref[i] for i in range(NZ)]
    count = {"z": 0, "s": 0}

    def opaque_zero():
        count["z"] += 1
        return zeros[count["z"] % NZ]

    lane = lax.broadcasted_iota(jnp.int32, (KB, 128), 1)
    row = lax.broadcasted_iota(jnp.int32, (KB, 128), 0)
    head = lax.broadcasted_iota(jnp.int32, (1, 128), 1) // DH
    wr_buf[...] = jnp.broadcast_to(wr_ref[...].astype(f32).reshape(1, D), (8, D))
    full = (0, D, 0, D)

    def ln_stage(b, g):
        for r in range(0, RC, LR):
            h = layernorm(get(x_buf, chunk_of(b, g, LR, r), ALL).astype(f32))
            put(x_buf, chunk_of(b + HB, g, LR, r), ALL, h)
            yield

    def qkv_stage(b, g):
        for t, dst in enumerate((q_buf, k_buf, v_buf)):
            y = jnp.dot(get(x_buf, rows_of(b + HB + opaque_zero()), ALL), get(wqkv_buf, full, g + t * G),
                        preferred_element_type=f32)
            put(dst, rows_of(b), g, y if t else y * (SCALE * LOG2E))
            yield

    def blockdiag(w):
        z = jnp.zeros_like(w)
        return pltpu.bitcast(jnp.concatenate([jnp.where(head == h, w, z) for h in range(4)], axis=0), bf16)

    def segment(x, op, fill):
        out = None
        for h in range(4):
            r = op(jnp.where(head == h, x, fill), axis=-1, keepdims=True)
            out = r if out is None else jnp.where(head == h, r, out)
        return out

    def att_stage(b, g, first=False):
        count["s"] ^= 1
        s_put, s_get = s_buf.at[count["s"]], s_buf.at[count["s"] + zeros[0]]
        causal = lane % KB <= row
        parts = []
        for i0 in range(0, NT, AQ):
            tiles = {u: range(max(i0, u - NT), min(i0 + AQ, u + 1))
                     for u in range(NT if first else i0, NT + i0 + AQ)}
            bz = b + zeros[i0 // AQ] if i0 else b
            s = {}
            for u, qs in tiles.items():
                su = lax.dot_general(get(q_buf, rows_of(b, len(qs) * KB, qs[0] * KB), g),
                                     blockdiag(words(k_buf, rows_of(bz, KB, (u - NT) * KB), g)),
                                     (((1,), (1,)), ((), ())), preferred_element_type=f32)
                for n, i in enumerate(qs):
                    s[u, i] = su[n * KB:(n + 1) * KB]
                if u - NT >= i0:
                    i = u - NT
                    s[u, i] = jnp.where(causal, s[u, i], NEG if first else s.pop((i, i)))
            m = {}
            for (u, i), t in s.items():
                s_put[u, i * KB:(i + 1) * KB, :] = t
                m[i] = jnp.maximum(m[i], t) if i in m else t
            parts.append((tiles, bz, {i: segment(t, jnp.max, -np.inf) for i, t in m.items()}))
        yield
        outs = []
        for tiles, bz, m in parts:
            diag, l, acc = {}, {}, {}

            def prob(u, i):
                if i in diag and u == i + NT:
                    return diag[i]
                e = jnp.exp2(s_get[u + NT if u == i else u, i * KB:(i + 1) * KB, :] - m[i])
                l[i] = l[i] + e if i in l else e
                if u != i:
                    return e
                diag[i] = jnp.where(causal, e, 0.0)
                return jnp.where(causal, 0.0, e)

            for u, qs in tiles.items():
                pu = jnp.concatenate([prob(u, i) for i in qs], axis=0).astype(bf16)
                ou = jnp.dot(pu, blockdiag(words(v_buf, rows_of(bz, KB, (u - NT) * KB), g)),
                             preferred_element_type=f32)
                for n, i in enumerate(qs):
                    t = ou[n * KB:(n + 1) * KB]
                    acc[i] = acc[i] + t if i in acc else t
            outs += [acc[i] * recip(segment(l[i], jnp.sum, 0.0)) for i in sorted(acc)]
            yield
        put(o_buf, rows_of(b), g, jnp.concatenate(outs, axis=0))

    def out_proj(b, n, off, cols):
        z = opaque_zero()
        a = jnp.dot(get(o_buf, rows_of(b + z, n, off), ALL),
                    get(wo_buf, (z, D, 0, D) if n < R else full, cols), preferred_element_type=f32)
        put(x1_buf, rows_of(b, n, off), cols, get(x_buf, rows_of(b + z, n, off), cols).astype(f32) + rb(a))

    def out_stage(b, g):
        out_proj(b, R, 0, g)
        yield

    def router(h):
        wr = jnp.concatenate([wr_buf[...]] * (h.shape[0] // 8), axis=0)
        return rb(jnp.sum(h * wr, axis=-1, keepdims=True))

    best = x_buf.bitcast(u32).at[:, pl.ds((HB + NB) * R // 2, ER)]

    def epi_stage(b, g, valid=None):
        src = b if valid is None else jnp.maximum(b, 0)
        dst = b if valid is None else jnp.where(valid, b, NB)
        for r0 in range(0, RC, ER):
            x1 = get(x1_buf, chunk_of(src, g, ER, r0), ALL).astype(f32)
            h1 = layernorm(x1)
            put(x1_buf, chunk_of(dst + HB, g, ER, r0), ALL, h1)
            h1 = rb(h1)
            put(x_buf, chunk_of(dst, g, ER, r0), ALL, x1 + h1)
            r = jnp.broadcast_to(router(h1), (ER, 128))
            if valid is not None:
                r = jnp.where(valid, r, -np.inf)
            bv = pltpu.bitcast(best[0], f32)
            best[0] = pltpu.bitcast(jnp.where(r > bv, r, bv), u32)
            best[1] = jnp.where(r > bv, pltpu.bitcast(row[:ER] + (b * R + g * RC + r0), u32), best[1])
            yield

    def ffn(xs):
        xs = jnp.broadcast_to(xs, (8, D))
        if XM:
            eye = lax.broadcasted_iota(jnp.int32, (128, 128), 0) == lax.broadcasted_iota(jnp.int32, (128, 128), 1)
            for c in range(0, D, 128):
                d = jnp.where(eye, jnp.concatenate([xs[:, c:c + 128]] * 16, axis=0), 0.0).astype(bf16)
                xcol_buf[c:c + 128, :] = jnp.dot(d, jnp.ones((128, 128), bf16), preferred_element_type=f32)
        else:
            for c in range(0, D, 128):
                xcol_buf[c:c + 128, :] = jnp.concatenate([xs[:, c:c + 128]] * 16, axis=0).T
        hb = xs.astype(bf16)

        def on_mxu(cols):
            return [jnp.dot(hb, get(w, full, cols), preferred_element_type=f32) for w in (wg_buf, wu_buf)]

        def on_vpu(cols):
            xcol = xcol_buf.at[pl.ds(pl.multiple_of(opaque_zero() * cols[0], 16), D)]
            acc = [0.0, 0.0]
            for k in range(0, D, 16):
                xk = jnp.concatenate([xcol[k:k + 16, :]] * len(cols), axis=1)
                for t, w in enumerate((wg_buf, wu_buf)):
                    prod = get(w, (0, D, k, 16), cols).astype(f32) * xk
                    acc[t] = (acc[t] + prod[:8]) + prod[8:]
            return [jnp.broadcast_to(jnp.sum(a, axis=0, keepdims=True), a.shape) for a in acc]

        def act(gate, up):
            gate = rb(gate)
            return (rb(gate * jax.nn.sigmoid(gate)) * rb(up)).astype(bf16)

        queue, c, y = [], 0, 0.0
        for t in FPLAN.split():
            cols = range(c, c + int(t[1:]))
            c += len(cols)
            if t[0] == "G":
                queue.append((cols, act(*on_mxu(cols))))
                continue
            cols, a = queue.pop(0) if t[0] == "D" else (cols, act(*on_vpu(cols)))
            y = y + jnp.dot(a, get(wd_buf, (0, F, cols[0] * 128, len(cols) * 128), ALL),
                            preferred_element_type=f32)
        assert c * 128 == F and not queue
        return rb(rb(y) * rb(jax.nn.sigmoid(router(xs))))

    def steps(name, order, unroll=G, pre=None, **stages):
        order = order.split()
        pair = 1 + any(t.isupper() for t in order)

        def body(j, _):
            if pre is not None:
                pre(j)
            for n in range(0, unroll, pair):
                live = {}
                for t in order:
                    key = (t.lower().replace("p", "a"), int(t.isupper()))
                    if key not in live:
                        live[key] = stages[key[0]](j * unroll + n + key[1])
                    next(live[key], None)
                assert all(next(gen, 1) == 1 for gen in live.values())
        if unroll == G:
            body(0, None)
        else:
            lax.fori_loop(0, G // unroll, body, None)

    P = functools.partial

    def stream_weights(j):
        pl.when(j + 1 < G // U_P1)(lambda: start(wqkv_copy(j + 1)))
        pl.when(j + 1 == G // U_P1)(lambda: start(x_copy(2) + wo_copy))
        wait(wqkv_copy(j))

    wait(x_copy(0))
    start(x_copy(1))
    for g in ALL:
        run(ln_stage(0, g))
    wait(x_copy(1))
    steps("P1", O_P1, U_P1, pre=stream_weights, q=P(qkv_stage, 0), l=P(ln_stage, 1))
    wait(x_copy(2))
    for b in range(3, NB):
        start(x_copy(b))

    def layer(li, _):
        best[0] = pltpu.bitcast(jnp.full((ER, 128), -np.inf, f32), u32)
        best[1] = jnp.zeros((ER, 128), u32)
        steps("P2", O_P2, U_P2, a=P(att_stage, 0, first=True), q=P(qkv_stage, 1), l=P(ln_stage, 2))

        @pl.when(li == 0)
        def _():
            wait(wo_copy)
            for b in range(3, NB):
                wait(x_copy(b))
            start(ffn_copy)

        def steady(b, _):
            steps("S", O_S, e=P(epi_stage, b - 2, valid=b >= 2), o=P(out_stage, b - 1), a=P(att_stage, b),
                  q=P(qkv_stage, (b + 1) & (NB - 1)), l=P(ln_stage, (b + 2) & (NB - 1)))
        lax.fori_loop(1, NB - li, steady, None)

        @pl.when(li == 1)
        def _():
            start(out_copy(0, (NB - 3) * R, 0))
            steps("E1", O_E1, U_E1, e=P(epi_stage, NB - 3), o=P(out_stage, NB - 2), a=P(att_stage, NB - 1))
            start(out_copy(NB - 3, R, 1))

        n_out = 0
        epi = (None for b in (NB - 2, NB - 1) for g in ALL for _ in epi_stage(b, g))
        for t in O_E2.split():
            if t[0] == "e":
                for _ in range(int(t[1:])):
                    next(epi)
            else:
                out_proj(NB - 1, int(t[1:]) * RC, n_out * RC, ALL)
                n_out += int(t[1:])
        run(epi)
        assert n_out == G

        pl.when(li == 0)(lambda: wait(ffn_copy))
        pl.when(li == 1)(lambda: start(out_copy(NB // 2 - 1, 2 * R, 2)))

        bv, bi = pltpu.bitcast(best[0], f32), pltpu.bitcast(best[1], jnp.int32).astype(f32)
        idx = jnp.min(jnp.where(bv == jnp.max(bv, axis=0, keepdims=True), bi, float(S - 1))).astype(jnp.int32)
        tile = lax.shift_right_logical(idx, 4)
        x1 = get(x1_buf, (tile, 16, 0, 16), ALL).astype(f32)
        h1 = get(x1_buf, (tile + HB * R // 16, 16, 0, 16), ALL).astype(f32)
        sel = lax.broadcasted_iota(jnp.int32, (16, D), 0) == idx - tile * 16
        y = ffn(jnp.sum(jnp.where(sel, h1, 0.0), axis=0, keepdims=True))
        new = rb(x1 + jnp.where(sel, rb(h1 + jnp.concatenate([y, y], axis=0)), h1))

        @pl.when(li == 0)
        def _():
            put(x_buf, (tile, 16, 0, 16), ALL, new)
            h = layernorm(new)
            put(x_buf, (tile + HB * R // 16, 16, 0, 16), ALL, h)

            @pl.when(idx < R)
            def _():
                for t, dst in enumerate((q_buf, k_buf, v_buf)):
                    y = jnp.dot(h.astype(bf16), get(wqkv_buf, full, range(t * G, (t + 1) * G)),
                                preferred_element_type=f32)
                    put(dst, (tile, 16, 0, 16), ALL, y if t else y * (SCALE * LOG2E))

        @pl.when(li == 1)
        def _():
            wait(out_copy(0, (NB - 3) * R, 0) + out_copy(NB - 3, R, 1) + out_copy(NB // 2 - 1, 2 * R, 2))
            put(x_buf, (tile, 16, 0, 16), ALL, new)
            start(out_copy(tile, 16, 0))
            wait(out_copy(tile, 16, 0))

    lax.fori_loop(0, 2, layer, None)


@jax.jit
def pallas_interleave_layers__sliding_block__moe_arch_mod__prompt_kernel(
    A_x, A_wqkv, A_wo, B_x, B_w_r, B_w_gate, B_w_up, B_w_down,
):
    any_spec = pl.BlockSpec(memory_space=pl.ANY)

    def tiled(rows, cols):
        return pltpu.VMEM((cols // 128, rows, 128), bf16)

    out = pl.pallas_call(
        kernel,
        out_shape=jax.ShapeDtypeStruct((S, D), bf16),
        in_specs=[any_spec, any_spec, any_spec, pl.BlockSpec(memory_space=pltpu.VMEM),
                  any_spec, any_spec, any_spec],
        out_specs=any_spec,
        scratch_shapes=[
            tiled((HB + NB) * R + 2 * RC, D),
            tiled(2 * HB * R, D),
            tiled(S, D), tiled(S, D), tiled(S, D), tiled(S, D),
            pltpu.VMEM((2, 2 * NT, R, 128), f32),
            tiled(D, 3 * D), tiled(D, D), tiled(D, F), tiled(D, F), tiled(F, D),
            pltpu.VMEM((8, D), f32),
            pltpu.VMEM((D, 128), f32),
            pltpu.SMEM((NZ,), jnp.int32),
            pltpu.SemaphoreType.DMA((NB,)),
            pltpu.SemaphoreType.DMA((G,)),
            pltpu.SemaphoreType.DMA((2,)),
            pltpu.SemaphoreType.DMA((3,)),
        ],
        compiler_params=pltpu.CompilerParams(
            vmem_limit_bytes=100 * 1024 * 1024, disable_bounds_checks=True,
            flags={"XLA_TPU_FORCE_LP_LLO_SCHEDULER": True}),
        name="kern",
    )(A_x.reshape(S, D), A_wqkv, A_wo, B_w_r, B_w_gate, B_w_up, B_w_down)
    return out.reshape(1, S, D)
```

```python
import functools
import numpy as np
import jax
import jax.numpy as jnp
from jax import lax
from jax.experimental import pallas as pl
from jax.experimental.pallas import tpu as pltpu

S, D, F = 2048, 1024, 3584
DH = 32
R = 256
NB = S // R
G = D // 128
RC = R // G
KB = 32
NT = R // KB
HB = NB + 1
f32, bf16, u32 = jnp.float32, jnp.bfloat16, jnp.uint32
LOG2E = 1.4426950408889634
SCALE = float(np.float32(DH ** -0.5).astype(bf16))
EPS = float(np.float32(1e-5).astype(bf16))
NEG = -1e9 * LOG2E
ALL = range(G)

AQ = 4
ER = 16
LR = 16
NZ = 6
XM = 0
O_P1 = "q l q l q"
O_P2 = "q l a q l p p q a"
O_S = "l o l a q e p q e p q a"
O_E1 = "e a o e p p a"
W0 = 0
U_P1 = 1
U_P2 = 2
U_E1 = 2
O_E2 = "o1 e4 o1 e4 o1 e4 o1 e4 o1 e4 o1 e4 o1 e2 o1"
FPLAN = "G2 G1 V1 G1 D0 V1 G1 D0 V1 G1 D0 V1 G1 D0 V1 G1 D0 V1 G1 D0 V1 G1 D0 V1 G1 D0 V1 G1 D0 V1 G1 D0 V1 G1 D0 V1 D0 V1 D0 V1"


def rb(x):
    return x.astype(bf16).astype(f32)


def recip(x):
    r = pl.reciprocal(x, approx=True)
    return r * (2.0 - x * r)


def layernorm(x):
    m = jnp.sum(x, axis=-1, keepdims=True) * (1.0 / D)
    mb = rb(m)
    c = x - mb
    v = jnp.sum(c * c, axis=-1, keepdims=True) * (1.0 / D) - (m - mb) * (m - mb)
    s = rb(jnp.sqrt(rb(rb(v) + EPS)))
    return rb(c) * recip(s)


def aligned(i, n):
    return pl.ds(i * n if isinstance(i, int) else pl.multiple_of(i * n, n), n)


def window(ref, rows, div):
    blk, span, off, n = rows
    return ref.at[:, aligned(blk, span // div)], pl.ds(off // div, n // div)


def put(ref, rows, cols, x):
    ref, rows = window(ref, rows, 1)
    for i, c in enumerate(cols if isinstance(cols, range) else [cols]):
        ref[c, rows, :] = x[:, i * 128:(i + 1) * 128].astype(bf16)


def words(ref, rows, cols):
    ref, rows = window(ref.bitcast(u32), rows, 2)
    return jnp.concatenate([ref[c, rows, :] for c in (cols if isinstance(cols, range) else [cols])], axis=1)


def get(ref, rows, cols):
    return pltpu.bitcast(words(ref, rows, cols), bf16)


def rows_of(b, n=R, off=0):
    return (b - 1, R, off + R, n) if off < 0 else (b, R, off, n)


def chunk_of(b, g, n=RC, off=0):
    return (b, R, g * RC + off, n) if isinstance(g, int) else (b * G + g, RC, off, n)


def start(copies):
    for c in copies:
        c.start()


def wait(copies):
    for c in copies:
        c.wait()


def run(gen):
    for _ in gen:
        pass


def kernel(x_hbm, wqkv_hbm, wo_hbm, wr_hbm, wg_hbm, wu_hbm, wd_hbm, out_hbm,
           x_buf, x1_buf, q_buf, k_buf, v_buf, o_buf, s_buf, wqkv_buf, wo_buf,
           wg_buf, wu_buf, wd_buf, wr_ref, wr_buf, xcol_buf, zero_ref, sem_q, sem_w, sem_o):
    def x_copy(rows, sem):
        return [pltpu.make_async_copy(x_hbm.at[rows, aligned(c, 128)], x_buf.at[c, rows], sem) for c in ALL]

    def out_copy(b, n, sem):
        return [pltpu.make_async_copy(x_buf.at[c, aligned(b, n)], out_hbm.at[aligned(b, n), aligned(c, 128)],
                                      sem_o.at[sem]) for c in ALL]

    def w_copy(src, dst, cols, sem):
        return [pltpu.make_async_copy(src.at[:, aligned(c, 128)], dst.at[c], sem) for c in cols]

    def head_copy(g):
        return (w_copy(wqkv_hbm, wqkv_buf, [g + t * G for t in range(3)], sem_q.at[g])
                + x_copy(aligned(G + g, RC), sem_q.at[g]) + x_copy(aligned(2 * G + g, RC), sem_q.at[g]))

    rest_copy = w_copy(wo_hbm, wo_buf, ALL, sem_w.at[0]) + x_copy(pl.ds(3 * R, S - 3 * R), sem_w.at[0]) + [pltpu.make_async_copy(wr_hbm, wr_ref, sem_w.at[0])]
    ffn_copy = (w_copy(wg_hbm, wg_buf, range(F // 128), sem_w.at[1])
                + w_copy(wu_hbm, wu_buf, range(F // 128), sem_w.at[1])
                + w_copy(wd_hbm, wd_buf, ALL, sem_w.at[1]))
    x0_copy = x_copy(pl.ds(0, R), sem_w.at[2])
    start(x0_copy)
    if W0 == 0:
        start(head_copy(0))

    for i in range(NZ):
        zero_ref[i] = 0
    zeros = [zero_ref[i] for i in range(NZ)]
    count = {"z": 0, "s": 0}

    def opaque_zero():
        count["z"] += 1
        return zeros[count["z"] % NZ]

    lane = lax.broadcasted_iota(jnp.int32, (KB, 128), 1)
    row = lax.broadcasted_iota(jnp.int32, (KB, 128), 0)
    head = lax.broadcasted_iota(jnp.int32, (1, 128), 1) // DH
    full = (0, D, 0, D)

    def ln_stage(b, g):
        for r in range(0, RC, LR):
            h = layernorm(get(x_buf, chunk_of(b, g, LR, r), ALL).astype(f32))
            put(x_buf, chunk_of(b + HB, g, LR, r), ALL, h)
            yield

    def qkv_stage(b, g):
        for t, dst in enumerate((q_buf, k_buf, v_buf)):
            y = jnp.dot(get(x_buf, rows_of(b + HB + opaque_zero()), ALL), get(wqkv_buf, full, g + t * G),
                        preferred_element_type=f32)
            put(dst, rows_of(b), g, y if t else y * (SCALE * LOG2E))
            yield

    def blockdiag(w):
        z = jnp.zeros_like(w)
        return pltpu.bitcast(jnp.concatenate([jnp.where(head == h, w, z) for h in range(4)], axis=0), bf16)

    def segment(x, op, fill):
        out = None
        for h in range(4):
            r = op(jnp.where(head == h, x, fill), axis=-1, keepdims=True)
            out = r if out is None else jnp.where(head == h, r, out)
        return out

    def att_stage(b, g, first=False):
        count["s"] ^= 1
        s_put, s_get = s_buf.at[count["s"]], s_buf.at[count["s"] + zeros[0]]
        causal = lane % KB <= row
        parts = []
        for i0 in range(0, NT, AQ):
            tiles = {u: range(max(i0, u - NT), min(i0 + AQ, u + 1))
                     for u in range(NT if first else i0, NT + i0 + AQ)}
            bz = b + zeros[i0 // AQ] if i0 else b
            s = {}
            for u, qs in tiles.items():
                su = lax.dot_general(get(q_buf, rows_of(b, len(qs) * KB, qs[0] * KB), g),
                                     blockdiag(words(k_buf, rows_of(bz, KB, (u - NT) * KB), g)),
                                     (((1,), (1,)), ((), ())), preferred_element_type=f32)
                for n, i in enumerate(qs):
                    s[u, i] = su[n * KB:(n + 1) * KB]
                if u - NT >= i0:
                    i = u - NT
                    s[u, i] = jnp.where(causal, s[u, i], NEG if first else s.pop((i, i)))
            m = {}
            for (u, i), t in s.items():
                s_put[u, i * KB:(i + 1) * KB, :] = t
                m[i] = jnp.maximum(m[i], t) if i in m else t
            parts.append((tiles, bz, {i: segment(t, jnp.max, -np.inf) for i, t in m.items()}))
        yield
        outs = []
        for tiles, bz, m in parts:
            diag, l, acc = {}, {}, {}

            def prob(u, i):
                if i in diag and u == i + NT:
                    return diag[i]
                e = jnp.exp2(s_get[u + NT if u == i else u, i * KB:(i + 1) * KB, :] - m[i])
                l[i] = l[i] + e if i in l else e
                if u != i:
                    return e
                diag[i] = jnp.where(causal, e, 0.0)
                return jnp.where(causal, 0.0, e)

            for u, qs in tiles.items():
                pu = jnp.concatenate([prob(u, i) for i in qs], axis=0).astype(bf16)
                ou = jnp.dot(pu, blockdiag(words(v_buf, rows_of(bz, KB, (u - NT) * KB), g)),
                             preferred_element_type=f32)
                for n, i in enumerate(qs):
                    t = ou[n * KB:(n + 1) * KB]
                    acc[i] = acc[i] + t if i in acc else t
            outs += [acc[i] * recip(segment(l[i], jnp.sum, 0.0)) for i in sorted(acc)]
            yield
        put(o_buf, rows_of(b), g, jnp.concatenate(outs, axis=0))

    def out_proj(b, n, off, cols):
        z = opaque_zero()
        a = jnp.dot(get(o_buf, rows_of(b + z, n, off), ALL),
                    get(wo_buf, (z, D, 0, D) if n < R else full, cols), preferred_element_type=f32)
        put(x1_buf, rows_of(b, n, off), cols, get(x_buf, rows_of(b + z, n, off), cols).astype(f32) + rb(a))

    def out_stage(b, g):
        out_proj(b, R, 0, g)
        yield

    def router(h):
        wr = jnp.concatenate([wr_buf[...]] * (h.shape[0] // 8), axis=0)
        return rb(jnp.sum(h * wr, axis=-1, keepdims=True))

    best = x_buf.bitcast(u32).at[:, pl.ds((HB + NB) * R // 2, ER)]

    def epi_stage(b, g, valid=None):
        src = b if valid is None else jnp.maximum(b, 0)
        dst = b if valid is None else jnp.where(valid, b, NB)
        for r0 in range(0, RC, ER):
            x1 = get(x1_buf, chunk_of(src, g, ER, r0), ALL).astype(f32)
            h1 = layernorm(x1)
            put(x1_buf, chunk_of(dst + HB, g, ER, r0), ALL, h1)
            h1 = rb(h1)
            put(x_buf, chunk_of(dst, g, ER, r0), ALL, x1 + h1)
            r = jnp.broadcast_to(router(h1), (ER, 128))
            if valid is not None:
                r = jnp.where(valid, r, -np.inf)
            bv = pltpu.bitcast(best[0], f32)
            best[0] = pltpu.bitcast(jnp.where(r > bv, r, bv), u32)
            best[1] = jnp.where(r > bv, pltpu.bitcast(row[:ER] + (b * R + g * RC + r0), u32), best[1])
            yield

    def ffn(xs):
        xs = jnp.broadcast_to(xs, (8, D))
        if XM:
            eye = lax.broadcasted_iota(jnp.int32, (128, 128), 0) == lax.broadcasted_iota(jnp.int32, (128, 128), 1)
            for c in range(0, D, 128):
                d = jnp.where(eye, jnp.concatenate([xs[:, c:c + 128]] * 16, axis=0), 0.0).astype(bf16)
                xcol_buf[c:c + 128, :] = jnp.dot(d, jnp.ones((128, 128), bf16), preferred_element_type=f32)
        else:
            for c in range(0, D, 128):
                xcol_buf[c:c + 128, :] = jnp.concatenate([xs[:, c:c + 128]] * 16, axis=0).T
        hb = xs.astype(bf16)

        def on_mxu(cols):
            return [jnp.dot(hb, get(w, full, cols), preferred_element_type=f32) for w in (wg_buf, wu_buf)]

        def on_vpu(cols):
            xcol = xcol_buf.at[pl.ds(pl.multiple_of(opaque_zero() * cols[0], 16), D)]
            acc = [0.0, 0.0]
            for k in range(0, D, 16):
                xk = jnp.concatenate([xcol[k:k + 16, :]] * len(cols), axis=1)
                for t, w in enumerate((wg_buf, wu_buf)):
                    prod = get(w, (0, D, k, 16), cols).astype(f32) * xk
                    acc[t] = (acc[t] + prod[:8]) + prod[8:]
            return [jnp.broadcast_to(jnp.sum(a, axis=0, keepdims=True), a.shape) for a in acc]

        def act(gate, up):
            gate = rb(gate)
            return (rb(gate * jax.nn.sigmoid(gate)) * rb(up)).astype(bf16)

        queue, c, y = [], 0, 0.0
        for t in FPLAN.split():
            cols = range(c, c + int(t[1:]))
            c += len(cols)
            if t[0] == "G":
                queue.append((cols, act(*on_mxu(cols))))
                continue
            cols, a = queue.pop(0) if t[0] == "D" else (cols, act(*on_vpu(cols)))
            y = y + jnp.dot(a, get(wd_buf, (0, F, cols[0] * 128, len(cols) * 128), ALL),
                            preferred_element_type=f32)
        assert c * 128 == F and not queue
        return rb(rb(y) * rb(jax.nn.sigmoid(router(xs))))

    def steps(name, order, unroll=G, **stages):
        order = order.split()
        pair = 1 + any(t.isupper() for t in order)

        def body(j, _):
            for n in range(0, unroll, pair):
                live = {}
                for t in order:
                    key = (t.lower().replace("p", "a"), int(t.isupper()))
                    if key not in live:
                        live[key] = stages[key[0]](j * unroll + n + key[1])
                    next(live[key], None)
                assert all(next(gen, 1) == 1 for gen in live.values())
        if unroll == G:
            body(0, None)
        else:
            lax.fori_loop(0, G // unroll, body, None)

    P = functools.partial

    def first_qkv(g):
        pl.when(g + 2 < G)(lambda: start(head_copy(g + 2)))
        wait(head_copy(g))
        yield from qkv_stage(0, g)

    put(x1_buf, rows_of(0), ALL, jnp.zeros((R, D), f32))
    if W0 == 1:
        start(head_copy(0))
    wait(x0_copy)
    start(head_copy(1))
    for g in ALL:
        run(ln_stage(0, g))
    steps("P1", O_P1, U_P1, q=first_qkv, l=P(ln_stage, 1))
    start(rest_copy)

    def layer(li, _):
        best[0] = pltpu.bitcast(jnp.full((ER, 128), -np.inf, f32), u32)
        best[1] = jnp.zeros((ER, 128), u32)
        steps("P2", O_P2, U_P2, a=P(att_stage, 0, first=True), q=P(qkv_stage, 1), l=P(ln_stage, 2))

        @pl.when(li == 0)
        def _():
            wait(rest_copy)
            wr_buf[...] = jnp.broadcast_to(wr_ref[...].astype(f32).reshape(1, D), (8, D))
            start(ffn_copy)

        def steady(b, _):
            steps("S", O_S, e=P(epi_stage, b - 2, valid=b >= 2), o=P(out_stage, b - 1), a=P(att_stage, b),
                  q=P(qkv_stage, (b + 1) & (NB - 1)), l=P(ln_stage, (b + 2) & (NB - 1)))
        lax.fori_loop(1, NB - li, steady, None)

        @pl.when(li == 1)
        def _():
            start(out_copy(0, (NB - 3) * R, 0))
            steps("E1", O_E1, U_E1, e=P(epi_stage, NB - 3), o=P(out_stage, NB - 2), a=P(att_stage, NB - 1))
            start(out_copy(NB - 3, R, 1))

        n_out = 0
        epi = (None for b in (NB - 2, NB - 1) for g in ALL for _ in epi_stage(b, g))
        for t in O_E2.split():
            if t[0] == "e":
                for _ in range(int(t[1:])):
                    next(epi)
            else:
                out_proj(NB - 1, int(t[1:]) * RC, n_out * RC, ALL)
                n_out += int(t[1:])
        run(epi)
        assert n_out == G

        pl.when(li == 0)(lambda: wait(ffn_copy))
        pl.when(li == 1)(lambda: start(out_copy(NB // 2 - 1, 2 * R, 2)))

        bv, bi = pltpu.bitcast(best[0], f32), pltpu.bitcast(best[1], jnp.int32).astype(f32)
        idx = jnp.min(jnp.where(bv == jnp.max(bv, axis=0, keepdims=True), bi, float(S - 1))).astype(jnp.int32)
        tile = lax.shift_right_logical(idx, 4)
        x1 = get(x1_buf, (tile, 16, 0, 16), ALL).astype(f32)
        h1 = get(x1_buf, (tile + HB * R // 16, 16, 0, 16), ALL).astype(f32)
        sel = lax.broadcasted_iota(jnp.int32, (16, D), 0) == idx - tile * 16
        y = ffn(jnp.sum(jnp.where(sel, h1, 0.0), axis=0, keepdims=True))
        new = rb(x1 + jnp.where(sel, rb(h1 + jnp.concatenate([y, y], axis=0)), h1))

        @pl.when(li == 0)
        def _():
            put(x_buf, (tile, 16, 0, 16), ALL, new)
            h = layernorm(new)
            put(x_buf, (tile + HB * R // 16, 16, 0, 16), ALL, h)

            @pl.when(idx < R)
            def _():
                for t, dst in enumerate((q_buf, k_buf, v_buf)):
                    y = jnp.dot(h.astype(bf16), get(wqkv_buf, full, range(t * G, (t + 1) * G)),
                                preferred_element_type=f32)
                    put(dst, (tile, 16, 0, 16), ALL, y if t else y * (SCALE * LOG2E))

        @pl.when(li == 1)
        def _():
            wait(out_copy(0, (NB - 3) * R, 0) + out_copy(NB - 3, R, 1) + out_copy(NB // 2 - 1, 2 * R, 2))
            put(x_buf, (tile, 16, 0, 16), ALL, new)
            start(out_copy(tile, 16, 0))
            wait(out_copy(tile, 16, 0))

    lax.fori_loop(0, 2, layer, None)


@jax.jit
def pallas_interleave_layers__sliding_block__moe_arch_mod__prompt_kernel(
    A_x, A_wqkv, A_wo, B_x, B_w_r, B_w_gate, B_w_up, B_w_down,
):
    any_spec = pl.BlockSpec(memory_space=pl.ANY)

    def tiled(rows, cols):
        return pltpu.VMEM((cols // 128, rows, 128), bf16)

    out = pl.pallas_call(
        kernel,
        out_shape=jax.ShapeDtypeStruct((S, D), bf16),
        in_specs=[any_spec] * 7,
        out_specs=any_spec,
        scratch_shapes=[
            tiled((HB + NB) * R + 2 * RC, D),
            tiled(2 * HB * R, D),
            tiled(S, D), tiled(S, D), tiled(S, D), tiled(S, D),
            pltpu.VMEM((2, 2 * NT, R, 128), f32),
            tiled(D, 3 * D), tiled(D, D), tiled(D, F), tiled(D, F), tiled(F, D),
            pltpu.VMEM((D,), bf16),
            pltpu.VMEM((8, D), f32),
            pltpu.VMEM((D, 128), f32),
            pltpu.SMEM((NZ,), jnp.int32),
            pltpu.SemaphoreType.DMA((G,)),
            pltpu.SemaphoreType.DMA((3,)),
            pltpu.SemaphoreType.DMA((3,)),
        ],
        compiler_params=pltpu.CompilerParams(
            vmem_limit_bytes=100 * 1024 * 1024, disable_bounds_checks=True,
            flags={"XLA_TPU_FORCE_LP_LLO_SCHEDULER": True}),
        name="kern",
    )(A_x.reshape(S, D), A_wqkv, A_wo, B_w_r, B_w_gate, B_w_up, B_w_down)
    return out.reshape(1, S, D)
```

```python
import functools

import jax
import jax.numpy as jnp
import numpy as np
from jax import lax
from jax.experimental import pallas as pl
from jax.experimental.pallas import tpu as pltpu

S, D, F = 2048, 1024, 3584
DH = 32
R = 256
NB = S // R
G = D // 128
RC = R // G
RP = 16
KB = 32
NT = R // KB
AQ = 4
HB = NB + 1
NZ = 6
ALL = range(G)
f32, bf16, i32, u32 = jnp.float32, jnp.bfloat16, jnp.int32, jnp.uint32
LOG2E = 1.4426950408889634
QSCALE = float(np.float32(DH ** -0.5).astype(bf16)) * LOG2E
MASKED = -1e9 * LOG2E
EPS = float(np.float32(1e-5).astype(bf16))
FFN_PLAN = "G2 G1 V1" + " G1 D0 V1" * 11 + " D0 V1 D0 V1"


def rb(x):
    return x.astype(bf16).astype(f32)


def recip(x):
    r = pl.reciprocal(x, approx=True)
    return r * (2.0 - x * r)


def layernorm(x):
    m = jnp.sum(x, axis=-1, keepdims=True) * (1.0 / D)
    mb = rb(m)
    c = x - mb
    v = jnp.sum(c * c, axis=-1, keepdims=True) * (1.0 / D) - (m - mb) * (m - mb)
    s = rb(jnp.sqrt(rb(rb(v) + EPS)))
    return rb(c) * jnp.where(s == np.inf, 0.0, recip(s))


def aligned(i, n):
    return pl.ds(i * n if isinstance(i, int) else pl.multiple_of(i * n, n), n)


def window(ref, rows, div):
    blk, span, off, n = rows
    return ref.at[:, aligned(blk, span // div)], pl.ds(off // div, n // div)


def put(ref, rows, cols, x):
    ref, rows = window(ref, rows, 1)
    for i, c in enumerate(cols if isinstance(cols, range) else [cols]):
        ref[c, rows, :] = x[:, i * 128:(i + 1) * 128].astype(bf16)


def words(ref, rows, cols):
    ref, rows = window(ref.bitcast(u32), rows, 2)
    return jnp.concatenate([ref[c, rows, :] for c in (cols if isinstance(cols, range) else [cols])], axis=1)


def get(ref, rows, cols):
    return pltpu.bitcast(words(ref, rows, cols), bf16)


def rows_of(b, n=R, off=0):
    return (b - 1, R, off + R, n) if off < 0 else (b, R, off, n)


def piece_of(b, g, off):
    return (b, R, g * RC + off, RP) if isinstance(g, int) else (b * G + g, RC, off, RP)


def start(copies):
    for c in copies:
        c.start()


def wait(copies):
    for c in copies:
        c.wait()


def run(gen):
    for _ in gen:
        pass


def sweep(order, unroll, **stages):
    def body(j, _):
        for n in range(unroll):
            live = {name: stage(j * unroll + n) for name, stage in stages.items()}
            for name in order.split():
                next(live[name], None)
            assert all(next(gen, 1) == 1 for gen in live.values())
    if unroll == G:
        body(0, None)
    else:
        lax.fori_loop(0, G // unroll, body, None)


def kernel(x_hbm, wqkv_hbm, wo_hbm, wr_hbm, wg_hbm, wu_hbm, wd_hbm, out_hbm,
           x_buf, x1_buf, q_buf, k_buf, v_buf, o_buf, s_buf, wqkv_buf, wo_buf,
           wg_buf, wu_buf, wd_buf, wr_raw, wr_buf, xcol_buf, zero_ref, sem_head, sem_in, sem_out):
    def x_copy(rows, sem):
        return [pltpu.make_async_copy(x_hbm.at[rows, aligned(c, 128)], x_buf.at[c, rows], sem) for c in ALL]

    def out_copy(b, n, sem):
        return [pltpu.make_async_copy(x_buf.at[c, aligned(b, n)], out_hbm.at[aligned(b, n), aligned(c, 128)],
                                      sem_out.at[sem]) for c in ALL]

    def w_copy(src, dst, cols, sem):
        return [pltpu.make_async_copy(src.at[:, aligned(c, 128)], dst.at[c], sem) for c in cols]

    def head_copy(g):
        return (w_copy(wqkv_hbm, wqkv_buf, [g + t * G for t in range(3)], sem_head.at[g])
                + x_copy(aligned(G + g, RC), sem_head.at[g]) + x_copy(aligned(2 * G + g, RC), sem_head.at[g]))

    x0_copy = x_copy(pl.ds(0, R), sem_in.at[0])
    rest_copy = (w_copy(wo_hbm, wo_buf, ALL, sem_in.at[1]) + x_copy(pl.ds(3 * R, S - 3 * R), sem_in.at[1])
                 + [pltpu.make_async_copy(wr_hbm, wr_raw, sem_in.at[1])])
    ffn_copy = (w_copy(wg_hbm, wg_buf, range(F // 128), sem_in.at[2])
                + w_copy(wu_hbm, wu_buf, range(F // 128), sem_in.at[2])
                + w_copy(wd_hbm, wd_buf, ALL, sem_in.at[2]))
    start(x0_copy)
    start(head_copy(0))

    for i in range(NZ):
        zero_ref[i] = 0
    zeros = [zero_ref[i] for i in range(NZ)]
    count = {"zero": 0, "slot": 0}

    def next_zero():
        count["zero"] += 1
        return zeros[count["zero"] % NZ]

    lane = lax.broadcasted_iota(i32, (KB, 128), 1)
    row = lax.broadcasted_iota(i32, (KB, 128), 0)
    head = lax.broadcasted_iota(i32, (1, 128), 1) // DH
    full = (0, D, 0, D)
    best = x_buf.bitcast(u32).at[:, pl.ds((HB + NB) * R // 2, RP)]

    def ln_stage(b, g):
        for r in range(0, RC, RP):
            h = layernorm(get(x_buf, piece_of(b, g, r), ALL).astype(f32))
            put(x_buf, piece_of(b + HB, g, r), ALL, h)
            yield

    def qkv_stage(b, g):
        for t, dst in enumerate((q_buf, k_buf, v_buf)):
            y = jnp.dot(get(x_buf, rows_of(b + HB + next_zero()), ALL), get(wqkv_buf, full, g + t * G),
                        preferred_element_type=f32)
            put(dst, rows_of(b), g, y if t else y * QSCALE)
            yield

    def blockdiag(w):
        z = jnp.zeros_like(w)
        return pltpu.bitcast(jnp.concatenate([jnp.where(head == h, w, z) for h in range(4)], axis=0), bf16)

    def per_head(x, op, fill):
        out = None
        for h in range(4):
            r = op(jnp.where(head == h, x, fill), axis=-1, keepdims=True)
            out = r if out is None else jnp.where(head == h, r, out)
        return out

    def att_stage(b, g, first=False):
        count["slot"] ^= 1
        s_put, s_get = s_buf.at[count["slot"]], s_buf.at[count["slot"] + zeros[0]]
        causal = lane % KB <= row
        parts = []
        for i0 in range(0, NT, AQ):
            tiles = {u: range(max(i0, u - NT), min(i0 + AQ, u + 1))
                     for u in range(NT if first else i0, NT + i0 + AQ)}
            bz = b + zeros[i0 // AQ] if i0 else b
            s = {}
            for u, qs in tiles.items():
                su = lax.dot_general(get(q_buf, rows_of(b, len(qs) * KB, qs[0] * KB), g),
                                     blockdiag(words(k_buf, rows_of(bz, KB, (u - NT) * KB), g)),
                                     (((1,), (1,)), ((), ())), preferred_element_type=f32)
                for n, i in enumerate(qs):
                    s[u, i] = su[n * KB:(n + 1) * KB]
                if u - NT >= i0:
                    i = u - NT
                    s[u, i] = jnp.where(causal, s[u, i], MASKED if first else s.pop((i, i)))
            m = {}
            for (u, i), t in s.items():
                s_put[u, i * KB:(i + 1) * KB, :] = t
                m[i] = jnp.maximum(m[i], t) if i in m else t
            parts.append((tiles, bz, {i: per_head(t, jnp.max, -np.inf) for i, t in m.items()}))
        yield
        outs = []
        for tiles, bz, m in parts:
            near, l, acc = {}, {}, {}

            def prob(u, i):
                if i in near and u == i + NT:
                    return near[i]
                e = jnp.exp2(s_get[u + NT if u == i else u, i * KB:(i + 1) * KB, :] - m[i])
                l[i] = l[i] + e if i in l else e
                if u != i:
                    return e
                near[i] = jnp.where(causal, e, 0.0)
                return jnp.where(causal, 0.0, e)

            for u, qs in tiles.items():
                pu = jnp.concatenate([prob(u, i) for i in qs], axis=0).astype(bf16)
                ou = jnp.dot(pu, blockdiag(words(v_buf, rows_of(bz, KB, (u - NT) * KB), g)),
                             preferred_element_type=f32)
                for n, i in enumerate(qs):
                    t = ou[n * KB:(n + 1) * KB]
                    acc[i] = acc[i] + t if i in acc else t
            outs += [acc[i] * recip(per_head(l[i], jnp.sum, 0.0)) for i in sorted(acc)]
            yield
        put(o_buf, rows_of(b), g, jnp.concatenate(outs, axis=0))

    def out_proj(b, n, off, cols):
        z = next_zero()
        a = jnp.dot(get(o_buf, rows_of(b + z, n, off), ALL),
                    get(wo_buf, (z, D, 0, D) if n < R else full, cols), preferred_element_type=f32)
        put(x1_buf, rows_of(b, n, off), cols, get(x_buf, rows_of(b + z, n, off), cols).astype(f32) + rb(a))

    def out_stage(b, g):
        out_proj(b, R, 0, g)
        yield

    def router(h):
        wr = jnp.concatenate([wr_buf[...]] * (h.shape[0] // 8), axis=0)
        return rb(jnp.sum(h * wr, axis=-1, keepdims=True))

    def route_stage(b, g, valid=None):
        src = b if valid is None else jnp.maximum(b, 0)
        dst = b if valid is None else jnp.where(valid, b, NB)
        for r0 in range(0, RC, RP):
            x1 = get(x1_buf, piece_of(src, g, r0), ALL).astype(f32)
            h1 = layernorm(x1)
            put(x1_buf, piece_of(dst + HB, g, r0), ALL, h1)
            h1 = rb(h1)
            put(x_buf, piece_of(dst, g, r0), ALL, x1 + h1)
            r = jnp.broadcast_to(router(h1), (RP, 128))
            if valid is not None:
                r = jnp.where(valid, r, -np.inf)
            top = pltpu.bitcast(best[0], f32)
            best[0] = pltpu.bitcast(jnp.where(r > top, r, top), u32)
            best[1] = jnp.where(r > top, pltpu.bitcast(row[:RP] + (b * R + g * RC + r0), u32), best[1])
            yield

    def ffn(xs):
        xs = jnp.broadcast_to(xs, (8, D))
        for c in range(0, D, 128):
            xcol_buf[c:c + 128, :] = jnp.concatenate([xs[:, c:c + 128]] * 16, axis=0).T
        hb = xs.astype(bf16)

        def on_mxu(cols):
            return [jnp.dot(hb, get(w, full, cols), preferred_element_type=f32) for w in (wg_buf, wu_buf)]

        def on_vpu(cols):
            xcol = xcol_buf.at[pl.ds(pl.multiple_of(next_zero() * cols[0], 16), D)]
            acc = [0.0, 0.0]
            for k in range(0, D, 16):
                xk = jnp.concatenate([xcol[k:k + 16, :]] * len(cols), axis=1)
                for t, w in enumerate((wg_buf, wu_buf)):
                    prod = get(w, (0, D, k, 16), cols).astype(f32) * xk
                    acc[t] = (acc[t] + prod[:8]) + prod[8:]
            return [jnp.broadcast_to(jnp.sum(a, axis=0, keepdims=True), a.shape) for a in acc]

        def act(gate, up):
            gate = rb(gate)
            return (rb(gate * jax.nn.sigmoid(gate)) * rb(up)).astype(bf16)

        queue, c, y = [], 0, 0.0
        for t in FFN_PLAN.split():
            cols = range(c, c + int(t[1:]))
            c += len(cols)
            if t[0] == "G":
                queue.append((cols, act(*on_mxu(cols))))
                continue
            cols, a = queue.pop(0) if t[0] == "D" else (cols, act(*on_vpu(cols)))
            y = y + jnp.dot(a, get(wd_buf, (0, F, cols[0] * 128, len(cols) * 128), ALL),
                            preferred_element_type=f32)
        assert c * 128 == F and not queue
        return rb(rb(y) * rb(jax.nn.sigmoid(router(xs))))

    P = functools.partial

    def first_qkv(g):
        pl.when(g + 2 < G)(lambda: start(head_copy(g + 2)))
        wait(head_copy(g))
        yield from qkv_stage(0, g)

    put(x1_buf, rows_of(0), ALL, jnp.zeros((R, D), f32))
    wait(x0_copy)
    start(head_copy(1))
    for g in ALL:
        run(ln_stage(0, g))
    sweep("q l q l q", 1, q=first_qkv, l=P(ln_stage, 1))
    start(rest_copy)

    def layer(li, _):
        dyn0 = lax.shift_right_logical(li, 1)
        best[0] = pltpu.bitcast(jnp.full((RP, 128), -np.inf, f32), u32)
        best[1] = jnp.zeros((RP, 128), u32)
        sweep("q l a q a l q a a", G, a=P(att_stage, 0, first=True), q=P(qkv_stage, 1), l=P(ln_stage, 2 + dyn0))

        @pl.when(li == 0)
        def _():
            wait(rest_copy)
            wr_buf[...] = jnp.broadcast_to(wr_raw[...].astype(f32).reshape(1, D), (8, D))
            start(ffn_copy)

        def steady(b, _):
            sweep("o l a q a q e a q e l a", G, o=P(out_stage, b - 1), l=P(ln_stage, (b + 2) & (NB - 1)),
                  a=P(att_stage, b), q=P(qkv_stage, (b + 1) & (NB - 1)), e=P(route_stage, b - 2, valid=b >= 2))
        lax.fori_loop(1, NB - li, steady, None)

        @pl.when(li == 1)
        def _():
            start(out_copy(0, (NB - 3) * R, 0))
            sweep("e a o e a a a", 2, e=P(route_stage, NB - 3), a=P(att_stage, NB - 1), o=P(out_stage, NB - 2))
            start(out_copy(NB - 3, R, 1))

        routes = (None for b in (NB - 2, NB - 1) for g in ALL for _ in route_stage(b, g))
        for g, n in enumerate((4, 4, 4, 4, 4, 4, 2, 6)):
            out_proj(NB - 1, RC, g * RC, ALL)
            for _ in range(n):
                next(routes)

        pl.when(li == 0)(lambda: wait(ffn_copy))
        pl.when(li == 1)(lambda: start(out_copy(NB // 2 - 1, 2 * R, 2)))

        top, top_row = pltpu.bitcast(best[0], f32), pltpu.bitcast(best[1], i32).astype(f32)
        idx = jnp.min(jnp.where(top == jnp.max(top, axis=0, keepdims=True), top_row, float(S - 1))).astype(i32)
        tile = lax.shift_right_logical(idx, 4)
        rows, ln_rows = (tile, 16, 0, 16), (tile + HB * R // 16, 16, 0, 16)
        x1 = get(x1_buf, rows, ALL).astype(f32)
        h1 = get(x1_buf, ln_rows, ALL).astype(f32)
        sel = lax.broadcasted_iota(i32, (16, D), 0) == idx - tile * 16
        y = ffn(jnp.sum(jnp.where(sel, h1, 0.0), axis=0, keepdims=True))
        new = rb(x1 + jnp.where(sel, rb(h1 + jnp.concatenate([y, y], axis=0)), h1))

        @pl.when(li == 0)
        def _():
            put(x_buf, rows, ALL, new)
            h = layernorm(new)
            put(x_buf, ln_rows, ALL, h)

            @pl.when(idx < R)
            def _():
                for t, dst in enumerate((q_buf, k_buf, v_buf)):
                    y = jnp.dot(h.astype(bf16), get(wqkv_buf, full, range(t * G, (t + 1) * G)),
                                preferred_element_type=f32)
                    put(dst, rows, ALL, y if t else y * QSCALE)

        @pl.when(li == 1)
        def _():
            wait(out_copy(0, (NB - 3) * R, 0) + out_copy(NB - 3, R, 1) + out_copy(NB // 2 - 1, 2 * R, 2))
            put(x_buf, rows, ALL, new)
            start(out_copy(tile, 16, 0))
            wait(out_copy(tile, 16, 0))

    lax.fori_loop(0, 2, layer, None)


@jax.jit
def pallas_interleave_layers__sliding_block__moe_arch_mod__prompt_kernel(
    A_x: jax.Array,
    A_wqkv: jax.Array,
    A_wo: jax.Array,
    B_x: jax.Array,
    B_w_r: jax.Array,
    B_w_gate: jax.Array,
    B_w_up: jax.Array,
    B_w_down: jax.Array,
):
    del B_x
    any_spec = pl.BlockSpec(memory_space=pl.ANY)

    def tiled(rows, cols):
        return pltpu.VMEM((cols // 128, rows, 128), bf16)

    out = pl.pallas_call(
        kernel,
        out_shape=jax.ShapeDtypeStruct((S, D), bf16),
        in_specs=[any_spec] * 7,
        out_specs=any_spec,
        scratch_shapes=[
            tiled((HB + NB) * R + 2 * RC, D),
            tiled(2 * HB * R, D),
            tiled(S, D), tiled(S, D), tiled(S, D), tiled(S, D),
            pltpu.VMEM((2, 2 * NT, R, 128), f32),
            tiled(D, 3 * D), tiled(D, D), tiled(D, F), tiled(D, F), tiled(F, D),
            pltpu.VMEM((D,), bf16),
            pltpu.VMEM((8, D), f32),
            pltpu.VMEM((D, 128), f32),
            pltpu.SMEM((NZ,), i32),
            pltpu.SemaphoreType.DMA((G,)),
            pltpu.SemaphoreType.DMA((3,)),
            pltpu.SemaphoreType.DMA((3,)),
        ],
        compiler_params=pltpu.CompilerParams(
            vmem_limit_bytes=100 * 1024 * 1024, disable_bounds_checks=True,
            flags={"XLA_TPU_FORCE_LP_LLO_SCHEDULER": True}),
        name="kern",
    )(A_x.reshape(S, D), A_wqkv, A_wo, B_w_r, B_w_gate, B_w_up, B_w_down)
    return out.reshape(1, S, D)
```

```python
import functools

import jax
import jax.numpy as jnp
import numpy as np
from jax import lax
from jax.experimental import pallas as pl
from jax.experimental.pallas import tpu as pltpu

S, D, F = 2048, 1024, 3584
DH = 32
R = 256
NB = S // R
G = D // 128
RC = R // G
RP = 16
KB = 32
NT = R // KB
AQ = 4
HB = NB + 1
NZ = 6
ALL = range(G)
f32, bf16, i32, u32 = jnp.float32, jnp.bfloat16, jnp.int32, jnp.uint32
LOG2E = 1.4426950408889634
QSCALE = float(np.float32(DH ** -0.5).astype(bf16)) * LOG2E
MASKED = -1e9 * LOG2E
EPS = float(np.float32(1e-5).astype(bf16))
FFN_PLAN = "G2 G2 V1" + " G1 D0 V1" * 10 + " G1 V1 D0 D0 D0 V1"
TAIL_PLAN = ((128, 0, 0, 2, 3), (128, 0, 2, 4, 3), (128, 0, 4, 6, 4), (128, 0, 6, 8, 4),
             (64, 128, 0, 4, 4), (64, 128, 4, 8, 4), (64, 192, 0, 4, 4), (64, 192, 4, 8, 6))


def rb(x):
    return x.astype(bf16).astype(f32)


def recip(x):
    r = pl.reciprocal(x, approx=True)
    return r * (2.0 - x * r)


def layernorm(x):
    m = jnp.sum(x, axis=-1, keepdims=True) * (1.0 / D)
    mb = rb(m)
    c = x - mb
    v = jnp.sum(c * c, axis=-1, keepdims=True) * (1.0 / D) - (m - mb) * (m - mb)
    s = rb(jnp.sqrt(rb(rb(v) + EPS)))
    return rb(c) * jnp.where(s == np.inf, 0.0, recip(s))


def aligned(i, n):
    return pl.ds(i * n if isinstance(i, int) else pl.multiple_of(i * n, n), n)


def window(ref, rows, div):
    blk, span, off, n = rows
    return ref.at[:, aligned(blk, span // div)], pl.ds(off // div, n // div)


def put(ref, rows, cols, x):
    ref, rows = window(ref, rows, 1)
    for i, c in enumerate(cols if isinstance(cols, range) else [cols]):
        ref[c, rows, :] = x[:, i * 128:(i + 1) * 128].astype(bf16)


def words(ref, rows, cols):
    ref, rows = window(ref.bitcast(u32), rows, 2)
    return jnp.concatenate([ref[c, rows, :] for c in (cols if isinstance(cols, range) else [cols])], axis=1)


def get(ref, rows, cols):
    return pltpu.bitcast(words(ref, rows, cols), bf16)


def rows_of(b, n=R, off=0):
    return (b - 1, R, off + R, n) if off < 0 else (b, R, off, n)


def piece_of(b, g, off):
    return (b, R, g * RC + off, RP) if isinstance(g, int) else (b * G + g, RC, off, RP)


def start(copies):
    for c in copies:
        c.start()


def wait(copies):
    for c in copies:
        c.wait()


def run(gen):
    for _ in gen:
        pass


def sweep(order, unroll, **stages):
    def body(j, _):
        for n in range(unroll):
            live = {name: stage(j * unroll + n) for name, stage in stages.items()}
            for name in order.split():
                next(live[name], None)
            assert all(next(gen, 1) == 1 for gen in live.values())
    if unroll == G:
        body(0, None)
    else:
        lax.fori_loop(0, G // unroll, body, None)


def kernel(x_hbm, wqkv_hbm, wo_hbm, wr_hbm, wg_hbm, wu_hbm, wd_hbm, out_hbm,
           x_buf, x1_buf, q_buf, k_buf, v_buf, o_buf, s_buf, wqkv_buf, wo_buf,
           wg_buf, wu_buf, wd_buf, wr_raw, wr_buf, xcol_buf, zero_ref, sem_head, sem_in, sem_out):
    def x_copy(rows, sem):
        return [pltpu.make_async_copy(x_hbm.at[rows, aligned(c, 128)], x_buf.at[c, rows], sem) for c in ALL]

    def out_copy(b, n, sem):
        return [pltpu.make_async_copy(x_buf.at[c, aligned(b, n)], out_hbm.at[aligned(b, n), aligned(c, 128)],
                                      sem_out.at[sem]) for c in ALL]

    def w_copy(src, dst, cols, sem):
        return [pltpu.make_async_copy(src.at[:, aligned(c, 128)], dst.at[c], sem) for c in cols]

    def head_copy(g):
        return (w_copy(wqkv_hbm, wqkv_buf, [g + t * G for t in range(3)], sem_head.at[g])
                + x_copy(aligned(G + g, RC), sem_head.at[g]) + x_copy(aligned(2 * G + g, RC), sem_head.at[g]))

    x0_copy = x_copy(pl.ds(0, R), sem_in.at[0])
    rest_copy = (w_copy(wo_hbm, wo_buf, ALL, sem_in.at[1]) + x_copy(pl.ds(3 * R, S - 3 * R), sem_in.at[1])
                 + [pltpu.make_async_copy(wr_hbm, wr_raw, sem_in.at[1])])
    ffn_copy = (w_copy(wg_hbm, wg_buf, range(F // 128), sem_in.at[2])
                + w_copy(wu_hbm, wu_buf, range(F // 128), sem_in.at[2])
                + w_copy(wd_hbm, wd_buf, ALL, sem_in.at[2]))
    start(x0_copy)
    start(head_copy(0))

    for i in range(NZ):
        zero_ref[i] = 0
    zeros = [zero_ref[i] for i in range(NZ)]
    count = {"zero": 0, "slot": 0}

    def next_zero():
        count["zero"] += 1
        return zeros[count["zero"] % NZ]

    lane = lax.broadcasted_iota(i32, (KB, 128), 1)
    row = lax.broadcasted_iota(i32, (KB, 128), 0)
    head = lax.broadcasted_iota(i32, (1, 128), 1) // DH
    full = (0, D, 0, D)
    best = x_buf.bitcast(u32).at[:, pl.ds((HB + NB) * R // 2, RP)]

    def ln_stage(b, g):
        for r in range(0, RC, RP):
            h = layernorm(get(x_buf, piece_of(b, g, r), ALL).astype(f32))
            put(x_buf, piece_of(b + HB, g, r), ALL, h)
            yield

    def qkv_stage(b, g):
        for t, dst in enumerate((q_buf, k_buf, v_buf)):
            y = jnp.dot(get(x_buf, rows_of(b + HB + next_zero()), ALL), get(wqkv_buf, full, g + t * G),
                        preferred_element_type=f32)
            put(dst, rows_of(b), g, y if t else y * QSCALE)
            yield

    def blockdiag(w):
        z = jnp.zeros_like(w)
        return pltpu.bitcast(jnp.concatenate([jnp.where(head == h, w, z) for h in range(4)], axis=0), bf16)

    def per_head(x, op, fill):
        out = None
        for h in range(4):
            r = op(jnp.where(head == h, x, fill), axis=-1, keepdims=True)
            out = r if out is None else jnp.where(head == h, r, out)
        return out

    def att_stage(b, g, first=False):
        count["slot"] ^= 1
        s_put, s_get = s_buf.at[count["slot"]], s_buf.at[count["slot"] + zeros[0]]
        causal = lane % KB <= row
        parts = []
        for i0 in range(0, NT, AQ):
            tiles = {u: range(max(i0, u - NT), min(i0 + AQ, u + 1))
                     for u in range(NT if first else i0, NT + i0 + AQ)}
            bz = b + zeros[i0 // AQ] if i0 else b
            s = {}
            for u, qs in tiles.items():
                su = lax.dot_general(get(q_buf, rows_of(b, len(qs) * KB, qs[0] * KB), g),
                                     blockdiag(words(k_buf, rows_of(bz, KB, (u - NT) * KB), g)),
                                     (((1,), (1,)), ((), ())), preferred_element_type=f32)
                for n, i in enumerate(qs):
                    s[u, i] = su[n * KB:(n + 1) * KB]
                if u - NT >= i0:
                    i = u - NT
                    s[u, i] = jnp.where(causal, s[u, i], MASKED if first else s.pop((i, i)))
            m = {}
            for (u, i), t in s.items():
                s_put[u, i * KB:(i + 1) * KB, :] = t
                m[i] = jnp.maximum(m[i], t) if i in m else t
            parts.append((tiles, bz, {i: per_head(t, jnp.max, -np.inf) for i, t in m.items()}))
        yield
        outs = []
        for tiles, bz, m in parts:
            near, l, acc = {}, {}, {}

            def prob(u, i):
                if i in near and u == i + NT:
                    return near[i]
                e = jnp.exp2(s_get[u + NT if u == i else u, i * KB:(i + 1) * KB, :] - m[i])
                l[i] = l[i] + e if i in l else e
                if u != i:
                    return e
                near[i] = jnp.where(causal, e, 0.0)
                return jnp.where(causal, 0.0, e)

            for u, qs in tiles.items():
                pu = jnp.concatenate([prob(u, i) for i in qs], axis=0).astype(bf16)
                ou = jnp.dot(pu, blockdiag(words(v_buf, rows_of(bz, KB, (u - NT) * KB), g)),
                             preferred_element_type=f32)
                for n, i in enumerate(qs):
                    t = ou[n * KB:(n + 1) * KB]
                    acc[i] = acc[i] + t if i in acc else t
            outs += [acc[i] * recip(per_head(l[i], jnp.sum, 0.0)) for i in sorted(acc)]
            yield
        put(o_buf, rows_of(b), g, jnp.concatenate(outs, axis=0))

    def out_proj(b, n, off, cols):
        z = next_zero()
        a = jnp.dot(get(o_buf, rows_of(b + z, n, off), ALL),
                    get(wo_buf, (z, D, 0, D) if n < R else full, cols), preferred_element_type=f32)
        put(x1_buf, rows_of(b, n, off), cols, get(x_buf, rows_of(b + z, n, off), cols).astype(f32) + rb(a))

    def out_stage(b, g):
        out_proj(b, R, 0, g)
        yield

    def router(h):
        wr = jnp.concatenate([wr_buf[...]] * (h.shape[0] // 8), axis=0)
        return rb(jnp.sum(h * wr, axis=-1, keepdims=True))

    def route_stage(b, g, valid=None, pin=0):
        src = b if valid is None else jnp.maximum(b, 0)
        dst = b if valid is None else jnp.where(valid, b, NB)
        for r0 in range(0, RC, RP):
            x1 = get(x1_buf, piece_of(src, g, r0), ALL).astype(f32)
            h1 = layernorm(x1)
            put(x1_buf, piece_of(dst + HB, g, r0), ALL, h1)
            h1 = rb(h1)
            put(x_buf, piece_of(dst + pin, g, r0), ALL, x1 + h1)
            r = jnp.broadcast_to(router(h1), (RP, 128))
            if valid is not None:
                r = jnp.where(valid, r, -np.inf)
            top = pltpu.bitcast(best[0], f32)
            best[0] = pltpu.bitcast(jnp.where(r > top, r, top), u32)
            best[1] = jnp.where(r > top, pltpu.bitcast(row[:RP] + (b * R + g * RC + r0), u32), best[1])
            yield

    def ffn(xs):
        xs = jnp.broadcast_to(xs, (8, D))
        for c in range(0, D, 128):
            xcol_buf[c:c + 128, :] = jnp.concatenate([xs[:, c:c + 128]] * 16, axis=0).T
        hb = xs.astype(bf16)

        def on_mxu(cols):
            return [jnp.dot(hb, get(w, full, cols), preferred_element_type=f32) for w in (wg_buf, wu_buf)]

        def on_vpu(cols):
            xcol = xcol_buf.at[pl.ds(pl.multiple_of(next_zero() * cols[0], 16), D)]
            acc = [0.0, 0.0]
            for k in range(0, D, 16):
                xk = jnp.concatenate([xcol[k:k + 16, :]] * len(cols), axis=1)
                for t, w in enumerate((wg_buf, wu_buf)):
                    prod = get(w, (0, D, k, 16), cols).astype(f32) * xk
                    acc[t] = (acc[t] + prod[:8]) + prod[8:]
            return [jnp.broadcast_to(jnp.sum(a, axis=0, keepdims=True), a.shape) for a in acc]

        def act(gate, up):
            gate = rb(gate)
            return (rb(gate * jax.nn.sigmoid(gate)) * rb(up)).astype(bf16)

        queue, c, y = [], 0, 0.0
        for t in FFN_PLAN.split():
            cols = range(c, c + int(t[1:]))
            c += len(cols)
            if t[0] == "G":
                queue.append((cols, act(*on_mxu(cols))))
                continue
            cols, a = queue.pop(0) if t[0] == "D" else (cols, act(*on_vpu(cols)))
            y = y + jnp.dot(a, get(wd_buf, (0, F, cols[0] * 128, len(cols) * 128), ALL),
                            preferred_element_type=f32)
        assert c * 128 == F and not queue
        return rb(rb(y) * rb(jax.nn.sigmoid(router(xs))))

    P = functools.partial

    def first_qkv(g):
        pl.when(g + 2 < G)(lambda: start(head_copy(g + 2)))
        wait(head_copy(g))
        yield from qkv_stage(0, g)

    put(x1_buf, rows_of(0), ALL, jnp.zeros((R, D), f32))
    wait(x0_copy)
    start(head_copy(1))
    for g in ALL:
        run(ln_stage(0, g))
    sweep("q l q l q", 1, q=first_qkv, l=P(ln_stage, 1))
    start(rest_copy)

    def layer(li, _):
        dyn0 = lax.shift_right_logical(li, 1)
        best[0] = pltpu.bitcast(jnp.full((RP, 128), -np.inf, f32), u32)
        best[1] = jnp.zeros((RP, 128), u32)
        sweep("q l a q a l q a a", G, a=P(att_stage, 0, first=True), q=P(qkv_stage, 1), l=P(ln_stage, 2 + dyn0))

        @pl.when(li == 0)
        def _():
            wait(rest_copy)
            wr_buf[...] = jnp.broadcast_to(wr_raw[...].astype(f32).reshape(1, D), (8, D))
            start(ffn_copy)

        def steady(b, _):
            sweep("o l a q a q e a q e l a", G, o=P(out_stage, b - 1), l=P(ln_stage, (b + 2) & (NB - 1)),
                  a=P(att_stage, b), q=P(qkv_stage, (b + 1) & (NB - 1)), e=P(route_stage, b - 2, valid=b >= 2))
        lax.fori_loop(1, NB - li, steady, None)

        @pl.when(li == 1)
        def _():
            start(out_copy(0, (NB - 3) * R, 0))
            sweep("e a o e a a a", 2, e=P(route_stage, NB - 3), a=P(att_stage, NB - 1), o=P(out_stage, NB - 2))
            start(out_copy(NB - 3, R, 1))

        routes = (None for b in (NB - 2, NB - 1) for g in ALL for _ in route_stage(b, g, pin=dyn0))
        for n, off, c0, c1, pieces in TAIL_PLAN:
            out_proj(NB - 1, n, off, range(c0, c1))
            for _ in range(pieces):
                next(routes)
        assert next(routes, 1) == 1

        pl.when(li == 0)(lambda: wait(ffn_copy))
        pl.when(li == 1)(lambda: start(out_copy(NB // 2 - 1, 2 * R, 2)))

        top, top_row = pltpu.bitcast(best[0], f32), pltpu.bitcast(best[1], i32).astype(f32)
        idx = jnp.min(jnp.where(top == jnp.max(top, axis=0, keepdims=True), top_row, float(S - 1))).astype(i32)
        tile = lax.shift_right_logical(idx, 4)
        rows, ln_rows = (tile, 16, 0, 16), (tile + HB * R // 16, 16, 0, 16)
        x1 = get(x1_buf, rows, ALL).astype(f32)
        h1 = get(x1_buf, ln_rows, ALL).astype(f32)
        sel = lax.broadcasted_iota(i32, (16, D), 0) == idx - tile * 16
        y = ffn(jnp.sum(jnp.where(sel, h1, 0.0), axis=0, keepdims=True))
        new = rb(x1 + jnp.where(sel, rb(h1 + jnp.concatenate([y, y], axis=0)), h1))

        @pl.when(li == 0)
        def _():
            put(x_buf, rows, ALL, new)
            h = layernorm(new)
            put(x_buf, ln_rows, ALL, h)

            @pl.when(idx < R)
            def _():
                for t, dst in enumerate((q_buf, k_buf, v_buf)):
                    y = jnp.dot(h.astype(bf16), get(wqkv_buf, full, range(t * G, (t + 1) * G)),
                                preferred_element_type=f32)
                    put(dst, rows, ALL, y if t else y * QSCALE)

        @pl.when(li == 1)
        def _():
            wait(out_copy(0, (NB - 3) * R, 0) + out_copy(NB - 3, R, 1) + out_copy(NB // 2 - 1, 2 * R, 2))
            put(x_buf, rows, ALL, new)
            start(out_copy(tile, 16, 0))
            wait(out_copy(tile, 16, 0))

    lax.fori_loop(0, 2, layer, None)


@jax.jit
def pallas_interleave_layers__sliding_block__moe_arch_mod__prompt_kernel(
    A_x: jax.Array,
    A_wqkv: jax.Array,
    A_wo: jax.Array,
    B_x: jax.Array,
    B_w_r: jax.Array,
    B_w_gate: jax.Array,
    B_w_up: jax.Array,
    B_w_down: jax.Array,
):
    del B_x
    any_spec = pl.BlockSpec(memory_space=pl.ANY)

    def tiled(rows, cols):
        return pltpu.VMEM((cols // 128, rows, 128), bf16)

    out = pl.pallas_call(
        kernel,
        out_shape=jax.ShapeDtypeStruct((S, D), bf16),
        in_specs=[any_spec] * 7,
        out_specs=any_spec,
        scratch_shapes=[
            tiled((HB + NB) * R + 2 * RC, D),
            tiled(2 * HB * R, D),
            tiled(S, D), tiled(S, D), tiled(S, D), tiled(S, D),
            pltpu.VMEM((2, 2 * NT, R, 128), f32),
            tiled(D, 3 * D), tiled(D, D), tiled(D, F), tiled(D, F), tiled(F, D),
            pltpu.VMEM((D,), bf16),
            pltpu.VMEM((8, D), f32),
            pltpu.VMEM((D, 128), f32),
            pltpu.SMEM((NZ,), i32),
            pltpu.SemaphoreType.DMA((G,)),
            pltpu.SemaphoreType.DMA((3,)),
            pltpu.SemaphoreType.DMA((3,)),
        ],
        compiler_params=pltpu.CompilerParams(
            vmem_limit_bytes=100 * 1024 * 1024, disable_bounds_checks=True,
            flags={"XLA_TPU_FORCE_LP_LLO_SCHEDULER": True}),
        name="kern",
    )(A_x.reshape(S, D), A_wqkv, A_wo, B_w_r, B_w_gate, B_w_up, B_w_down)
    return out.reshape(1, S, D)
```

```python
import functools

import jax
import jax.numpy as jnp
import numpy as np
from jax import lax
from jax.experimental import pallas as pl
from jax.experimental.pallas import tpu as pltpu

S, D, F = 2048, 1024, 3584
DH = 32
R = 256
NB = S // R
G = D // 128
RC = R // G
RP = 16
KB = 32
NT = R // KB
AQ = 4
HB = NB + 1
NZ = 6
ALL = range(G)
f32, bf16, i32, u32 = jnp.float32, jnp.bfloat16, jnp.int32, jnp.uint32
LOG2E = 1.4426950408889634
QSCALE = float(np.float32(DH ** -0.5).astype(bf16)) * LOG2E
MASKED = -1e9 * LOG2E
EPS = float(np.float32(1e-5).astype(bf16))
FFN_PLAN = "G2 G2 V1" + " G1 D0 V1" * 10 + " G1 V1 D0 D0 D0 V1"
TAIL_PLAN = ((128, 0, 0, 2, 3), (128, 0, 2, 4, 3), (128, 0, 4, 6, 4), (128, 0, 6, 8, 4),
             (64, 128, 0, 4, 4), (64, 128, 4, 8, 4), (64, 192, 0, 4, 4), (64, 192, 4, 8, 6))


def rb(x):
    return x.astype(bf16).astype(f32)


def recip(x):
    r = pl.reciprocal(x, approx=True)
    return r * (2.0 - x * r)


def layernorm(x):
    m = jnp.sum(x, axis=-1, keepdims=True) * (1.0 / D)
    mb = rb(m)
    c = x - mb
    v = jnp.sum(c * c, axis=-1, keepdims=True) * (1.0 / D) - (m - mb) * (m - mb)
    s = rb(jnp.sqrt(rb(rb(v) + EPS)))
    return rb(c) * jnp.where(s == np.inf, 0.0, recip(s))


def aligned(i, n):
    return pl.ds(i * n if isinstance(i, int) else pl.multiple_of(i * n, n), n)


def window(ref, rows, div):
    blk, span, off, n = rows
    return ref.at[:, aligned(blk, span // div)], pl.ds(off // div, n // div)


def put(ref, rows, cols, x):
    ref, rows = window(ref, rows, 1)
    for i, c in enumerate(cols if isinstance(cols, range) else [cols]):
        ref[c, rows, :] = x[:, i * 128:(i + 1) * 128].astype(bf16)


def words(ref, rows, cols):
    ref, rows = window(ref.bitcast(u32), rows, 2)
    return jnp.concatenate([ref[c, rows, :] for c in (cols if isinstance(cols, range) else [cols])], axis=1)


def get(ref, rows, cols):
    return pltpu.bitcast(words(ref, rows, cols), bf16)


def rows_of(b, n=R, off=0):
    return (b - 1, R, off + R, n) if off < 0 else (b, R, off, n)


def piece_of(b, g, off):
    return (b, R, g * RC + off, RP) if isinstance(g, int) else (b * G + g, RC, off, RP)


def start(copies):
    for c in copies:
        c.start()


def wait(copies):
    for c in copies:
        c.wait()


def run(gen):
    for _ in gen:
        pass


def sweep(order, unroll, **stages):
    def body(j, _):
        for n in range(unroll):
            live = {name: stage(j * unroll + n) for name, stage in stages.items()}
            for name in order.split():
                next(live[name], None)
            assert all(next(gen, 1) == 1 for gen in live.values())
    if unroll == G:
        body(0, None)
    else:
        lax.fori_loop(0, G // unroll, body, None)


def kernel(x_hbm, wqkv_hbm, wo_hbm, wr_hbm, wg_hbm, wu_hbm, wd_hbm, out_hbm,
           x_buf, x1_buf, q_buf, k_buf, v_buf, o_buf, s_buf, wqkv_buf, wo_buf,
           wg_buf, wu_buf, wd_buf, wr_raw, wr_buf, xcol_buf, zero_ref, sem_head, sem_in, sem_out):
    def x_copy(rows, sem):
        return [pltpu.make_async_copy(x_hbm.at[rows, aligned(c, 128)], x_buf.at[c, rows], sem) for c in ALL]

    def out_copy(b, n, sem):
        return [pltpu.make_async_copy(x_buf.at[c, aligned(b, n)], out_hbm.at[aligned(b, n), aligned(c, 128)],
                                      sem_out.at[sem]) for c in ALL]

    def w_copy(src, dst, cols, sem):
        return [pltpu.make_async_copy(src.at[:, aligned(c, 128)], dst.at[c], sem) for c in cols]

    def head_copy(g):
        return (w_copy(wqkv_hbm, wqkv_buf, [g + t * G for t in range(3)], sem_head.at[g])
                + x_copy(aligned(G + g, RC), sem_head.at[g]) + x_copy(aligned(2 * G + g, RC), sem_head.at[g]))

    x0_copy = x_copy(pl.ds(0, R), sem_in.at[0])
    rest_copy = (w_copy(wo_hbm, wo_buf, ALL, sem_in.at[1]) + x_copy(pl.ds(3 * R, S - 3 * R), sem_in.at[1])
                 + [pltpu.make_async_copy(wr_hbm, wr_raw, sem_in.at[1])])
    ffn_copy = (w_copy(wg_hbm, wg_buf, range(F // 128), sem_in.at[2])
                + w_copy(wu_hbm, wu_buf, range(F // 128), sem_in.at[2])
                + w_copy(wd_hbm, wd_buf, ALL, sem_in.at[2]))
    start(x0_copy)
    start(head_copy(0))

    for i in range(NZ):
        zero_ref[i] = 0
    zeros = [zero_ref[i] for i in range(NZ)]
    count = {"zero": 0, "slot": 0}

    def next_zero():
        count["zero"] += 1
        return zeros[count["zero"] % NZ]

    lane = lax.broadcasted_iota(i32, (KB, 128), 1)
    row = lax.broadcasted_iota(i32, (KB, 128), 0)
    head = lax.broadcasted_iota(i32, (1, 128), 1) // DH
    full = (0, D, 0, D)
    best = x_buf.bitcast(u32).at[:, pl.ds((HB + NB) * R // 2, RP)]

    def ln_stage(b, g):
        for r in range(0, RC, RP):
            h = layernorm(get(x_buf, piece_of(b, g, r), ALL).astype(f32))
            put(x_buf, piece_of(b + HB, g, r), ALL, h)
            yield

    def qkv_stage(b, g):
        for t, dst in enumerate((q_buf, k_buf, v_buf)):
            y = jnp.dot(get(x_buf, rows_of(b + HB + next_zero()), ALL), get(wqkv_buf, full, g + t * G),
                        preferred_element_type=f32)
            put(dst, rows_of(b), g, y if t else y * QSCALE)
            yield

    def blockdiag(w):
        z = jnp.zeros_like(w)
        return pltpu.bitcast(jnp.concatenate([jnp.where(head == h, w, z) for h in range(4)], axis=0), bf16)

    def per_head(tiles, reduce):
        t = jnp.concatenate([tiles[i] for i in sorted(tiles)], axis=0).T
        t = jnp.concatenate([jnp.broadcast_to(reduce(t[h * DH:(h + 1) * DH]), (DH, AQ * KB))
                             for h in range(4)], axis=0).T
        return {i: t[n * KB:(n + 1) * KB] for n, i in enumerate(sorted(tiles))}

    def att_stage(b, g, first=False):
        count["slot"] ^= 1
        s_put, s_get = s_buf.at[count["slot"]], s_buf.at[count["slot"] + zeros[0]]
        causal = lane % KB <= row
        parts = []
        for i0 in range(0, NT, AQ):
            tiles = {u: range(max(i0, u - NT), min(i0 + AQ, u + 1))
                     for u in range(NT if first else i0, NT + i0 + AQ)}
            bz = b + zeros[i0 // AQ] if i0 else b
            s = {}
            for u, qs in tiles.items():
                su = lax.dot_general(get(q_buf, rows_of(b, len(qs) * KB, qs[0] * KB), g),
                                     blockdiag(words(k_buf, rows_of(bz, KB, (u - NT) * KB), g)),
                                     (((1,), (1,)), ((), ())), preferred_element_type=f32)
                for n, i in enumerate(qs):
                    s[u, i] = su[n * KB:(n + 1) * KB]
                if u - NT >= i0:
                    i = u - NT
                    s[u, i] = jnp.where(causal, s[u, i], MASKED if first else s.pop((i, i)))
            m = {}
            for (u, i), t in s.items():
                s_put[u, i * KB:(i + 1) * KB, :] = t
                m[i] = jnp.maximum(m[i], t) if i in m else t
            parts.append((tiles, bz, per_head(m, lambda t: jnp.max(t, axis=0, keepdims=True))))
        yield
        outs = []
        for tiles, bz, m in parts:
            near, l, acc = {}, {}, {}

            def prob(u, i):
                if i in near and u == i + NT:
                    return near[i]
                e = jnp.exp2(s_get[u + NT if u == i else u, i * KB:(i + 1) * KB, :] - m[i])
                l[i] = l[i] + e if i in l else e
                if u != i:
                    return e
                near[i] = jnp.where(causal, e, 0.0)
                return jnp.where(causal, 0.0, e)

            for u, qs in tiles.items():
                pu = jnp.concatenate([prob(u, i) for i in qs], axis=0).astype(bf16)
                ou = jnp.dot(pu, blockdiag(words(v_buf, rows_of(bz, KB, (u - NT) * KB), g)),
                             preferred_element_type=f32)
                for n, i in enumerate(qs):
                    t = ou[n * KB:(n + 1) * KB]
                    acc[i] = acc[i] + t if i in acc else t
            inv = per_head(l, lambda t: recip(jnp.sum(t, axis=0, keepdims=True)))
            outs += [acc[i] * inv[i] for i in sorted(acc)]
            yield
        put(o_buf, rows_of(b), g, jnp.concatenate(outs, axis=0))

    def out_proj(b, n, off, cols):
        z = next_zero()
        a = jnp.dot(get(o_buf, rows_of(b + z, n, off), ALL),
                    get(wo_buf, (z, D, 0, D) if n < R else full, cols), preferred_element_type=f32)
        put(x1_buf, rows_of(b, n, off), cols, get(x_buf, rows_of(b + z, n, off), cols).astype(f32) + rb(a))

    def out_stage(b, g):
        out_proj(b, R, 0, g)
        yield

    def router(h):
        wr = jnp.concatenate([wr_buf[...]] * (h.shape[0] // 8), axis=0)
        return rb(jnp.sum(h * wr, axis=-1, keepdims=True))

    def route_stage(b, g, valid=None, pin=0):
        src = b if valid is None else jnp.maximum(b, 0)
        dst = b if valid is None else jnp.where(valid, b, NB)
        for r0 in range(0, RC, RP):
            x1 = get(x1_buf, piece_of(src, g, r0), ALL).astype(f32)
            h1 = layernorm(x1)
            put(x1_buf, piece_of(dst + HB, g, r0), ALL, h1)
            h1 = rb(h1)
            put(x_buf, piece_of(dst + pin, g, r0), ALL, x1 + h1)
            r = jnp.broadcast_to(router(h1), (RP, 128))
            if valid is not None:
                r = jnp.where(valid, r, -np.inf)
            top = pltpu.bitcast(best[0], f32)
            best[0] = pltpu.bitcast(jnp.where(r > top, r, top), u32)
            best[1] = jnp.where(r > top, pltpu.bitcast(row[:RP] + (b * R + g * RC + r0), u32), best[1])
            yield

    def ffn(xs):
        xs = jnp.broadcast_to(xs, (8, D))
        for c in range(0, D, 128):
            xcol_buf[c:c + 128, :] = jnp.concatenate([xs[:, c:c + 128]] * 16, axis=0).T
        hb = xs.astype(bf16)

        def on_mxu(cols):
            return [jnp.dot(hb, get(w, full, cols), preferred_element_type=f32) for w in (wg_buf, wu_buf)]

        def on_vpu(cols):
            xcol = xcol_buf.at[pl.ds(pl.multiple_of(next_zero() * cols[0], 16), D)]
            acc = [0.0, 0.0]
            for k in range(0, D, 16):
                xk = jnp.concatenate([xcol[k:k + 16, :]] * len(cols), axis=1)
                for t, w in enumerate((wg_buf, wu_buf)):
                    prod = get(w, (0, D, k, 16), cols).astype(f32) * xk
                    acc[t] = (acc[t] + prod[:8]) + prod[8:]
            return [jnp.broadcast_to(jnp.sum(a, axis=0, keepdims=True), a.shape) for a in acc]

        def act(gate, up):
            gate = rb(gate)
            return (rb(gate * jax.nn.sigmoid(gate)) * rb(up)).astype(bf16)

        queue, c, y = [], 0, 0.0
        for t in FFN_PLAN.split():
            cols = range(c, c + int(t[1:]))
            c += len(cols)
            if t[0] == "G":
                queue.append((cols, act(*on_mxu(cols))))
                continue
            cols, a = queue.pop(0) if t[0] == "D" else (cols, act(*on_vpu(cols)))
            y = y + jnp.dot(a, get(wd_buf, (0, F, cols[0] * 128, len(cols) * 128), ALL),
                            preferred_element_type=f32)
        assert c * 128 == F and not queue
        return rb(rb(y) * rb(jax.nn.sigmoid(router(xs))))

    P = functools.partial

    def first_qkv(g):
        pl.when(g + 2 < G)(lambda: start(head_copy(g + 2)))
        wait(head_copy(g))
        yield from qkv_stage(0, g)

    put(x1_buf, rows_of(0), ALL, jnp.zeros((R, D), f32))
    wait(x0_copy)
    start(head_copy(1))
    for g in ALL:
        run(ln_stage(0, g))
    sweep("q l q l q", 1, q=first_qkv, l=P(ln_stage, 1))
    start(rest_copy)

    def layer(li, _):
        dyn0 = lax.shift_right_logical(li, 1)
        best[0] = pltpu.bitcast(jnp.full((RP, 128), -np.inf, f32), u32)
        best[1] = jnp.zeros((RP, 128), u32)
        sweep("q l a q a l q a a", G, a=P(att_stage, 0, first=True), q=P(qkv_stage, 1), l=P(ln_stage, 2 + dyn0))

        @pl.when(li == 0)
        def _():
            wait(rest_copy)
            wr_buf[...] = jnp.broadcast_to(wr_raw[...].astype(f32).reshape(1, D), (8, D))
            start(ffn_copy)

        def steady(b, _):
            sweep("l o l a q e a q e a q a", G, o=P(out_stage, b - 1), l=P(ln_stage, (b + 2) & (NB - 1)),
                  a=P(att_stage, b), q=P(qkv_stage, (b + 1) & (NB - 1)), e=P(route_stage, b - 2, valid=b >= 2))
        lax.fori_loop(1, NB - li, steady, None)

        @pl.when(li == 1)
        def _():
            start(out_copy(0, (NB - 3) * R, 0))
            sweep("e a o e a a a", 2, e=P(route_stage, NB - 3), a=P(att_stage, NB - 1), o=P(out_stage, NB - 2))
            start(out_copy(NB - 3, R, 1))

        routes = (None for b in (NB - 2, NB - 1) for g in ALL for _ in route_stage(b, g, pin=dyn0))
        for n, off, c0, c1, pieces in TAIL_PLAN:
            out_proj(NB - 1, n, off, range(c0, c1))
            for _ in range(pieces):
                next(routes)
        assert next(routes, 1) == 1

        pl.when(li == 0)(lambda: wait(ffn_copy))
        pl.when(li == 1)(lambda: start(out_copy(NB // 2 - 1, 2 * R, 2)))

        top, top_row = pltpu.bitcast(best[0], f32), pltpu.bitcast(best[1], i32).astype(f32)
        idx = jnp.min(jnp.where(top == jnp.max(top, axis=0, keepdims=True), top_row, float(S - 1))).astype(i32)
        tile = lax.shift_right_logical(idx, 4)
        rows, ln_rows = (tile, 16, 0, 16), (tile + HB * R // 16, 16, 0, 16)
        x1 = get(x1_buf, rows, ALL).astype(f32)
        h1 = get(x1_buf, ln_rows, ALL).astype(f32)
        sel = lax.broadcasted_iota(i32, (16, D), 0) == idx - tile * 16
        y = ffn(jnp.sum(jnp.where(sel, h1, 0.0), axis=0, keepdims=True))
        new = rb(x1 + jnp.where(sel, rb(h1 + jnp.concatenate([y, y], axis=0)), h1))

        @pl.when(li == 0)
        def _():
            put(x_buf, rows, ALL, new)
            h = layernorm(new)
            put(x_buf, ln_rows, ALL, h)

            @pl.when(idx < R)
            def _():
                for t, dst in enumerate((q_buf, k_buf, v_buf)):
                    y = jnp.dot(h.astype(bf16), get(wqkv_buf, full, range(t * G, (t + 1) * G)),
                                preferred_element_type=f32)
                    put(dst, rows, ALL, y if t else y * QSCALE)

        @pl.when(li == 1)
        def _():
            wait(out_copy(0, (NB - 3) * R, 0) + out_copy(NB - 3, R, 1) + out_copy(NB // 2 - 1, 2 * R, 2))
            put(x_buf, rows, ALL, new)
            start(out_copy(tile, 16, 0))
            wait(out_copy(tile, 16, 0))

    lax.fori_loop(0, 2, layer, None)


@jax.jit
def pallas_interleave_layers__sliding_block__moe_arch_mod__prompt_kernel(
    A_x: jax.Array,
    A_wqkv: jax.Array,
    A_wo: jax.Array,
    B_x: jax.Array,
    B_w_r: jax.Array,
    B_w_gate: jax.Array,
    B_w_up: jax.Array,
    B_w_down: jax.Array,
):
    del B_x
    any_spec = pl.BlockSpec(memory_space=pl.ANY)

    def tiled(rows, cols):
        return pltpu.VMEM((cols // 128, rows, 128), bf16)

    out = pl.pallas_call(
        kernel,
        out_shape=jax.ShapeDtypeStruct((S, D), bf16),
        in_specs=[any_spec] * 7,
        out_specs=any_spec,
        scratch_shapes=[
            tiled((HB + NB) * R + 2 * RC, D),
            tiled(2 * HB * R, D),
            tiled(S, D), tiled(S, D), tiled(S, D), tiled(S, D),
            pltpu.VMEM((2, 2 * NT, R, 128), f32),
            tiled(D, 3 * D), tiled(D, D), tiled(D, F), tiled(D, F), tiled(F, D),
            pltpu.VMEM((D,), bf16),
            pltpu.VMEM((8, D), f32),
            pltpu.VMEM((D, 128), f32),
            pltpu.SMEM((NZ,), i32),
            pltpu.SemaphoreType.DMA((G,)),
            pltpu.SemaphoreType.DMA((3,)),
            pltpu.SemaphoreType.DMA((3,)),
        ],
        compiler_params=pltpu.CompilerParams(
            vmem_limit_bytes=100 * 1024 * 1024, disable_bounds_checks=True,
            flags={"XLA_TPU_FORCE_LP_LLO_SCHEDULER": True}),
        name="kern",
    )(A_x.reshape(S, D), A_wqkv, A_wo, B_w_r, B_w_gate, B_w_up, B_w_down)
    return out.reshape(1, S, D)
```
